```python
import jax
import jax.numpy as jnp

def _softmax(x, axis=-1):
    return jax.nn.softmax(x, axis=axis)
def _gelu(x):
    return jax.nn.gelu(x, approximate=True)
def _silu(x):
    return jax.nn.silu(x)
def _sigmoid(x):
    return jax.nn.sigmoid(x)
def _layernorm(x, axis=-1, eps=1e-5):
    m = jnp.mean(x, axis=axis, keepdims=True)
    v = jnp.var(x, axis=axis, keepdims=True)
    return (x - m) / jnp.sqrt(v + eps)
def _scatter_add(tgt, idx, src, axis=0):
    return tgt.at[idx].add(src)
def _segment_sum(src, seg, n):
    return jax.ops.segment_sum(src, seg, n)
class _Rng:
    def __init__(self, key):
        self._k = key
    def _next(self):
        self._k, sub = jax.random.split(self._k)
        return sub
    def normal(self, shape):
        return jax.random.normal(self._next(), shape, dtype=jnp.bfloat16)
    def randint(self, lo, hi, shape):
        return jax.random.randint(self._next(), shape, lo, hi, dtype=jnp.int32)
    def uniform(self, shape, lo=0.0, hi=1.0):
        return jax.random.uniform(self._next(), shape, jnp.bfloat16, lo, hi)
    def permutation(self, n):
        return jax.random.permutation(self._next(), n)


kernel_name = 'recurrent_scan__sliding_local_dilated__glu_gated_swiglu__prompt'

def setup_inputs():
    _rng = _Rng(jax.random.key(int.from_bytes(__import__("os").urandom(4), "little")))
    _w = (lambda a: (lambda t: t.astype(jnp.bfloat16) if jnp.issubdtype(t.dtype, jnp.floating) else t)(jnp.asarray(a)))
    def _A_setup():
        B, S, D = 1, 2048, 1024
        return {
            "x": _w((lambda *s: _rng.normal(s) * 0.05)(B, S, D)),
            "wqkv": _w((lambda *s: _rng.normal(s) * 0.05)(D, 3 * D)),
            "wo": _w((lambda *s: _rng.normal(s) * 0.05)(D, D)),
        }
    _A_in = _A_setup()

    def _B_setup():
        B, S, D, F = 1, 2048, 1024, 3584
        return {
            "x": _w((lambda *s: _rng.normal(s) * 0.05)(B, S, D)),
            "w1": _w((lambda *s: _rng.normal(s) * 0.05)(D, F) * (2.0 / D) ** 0.5),
            "w3": _w((lambda *s: _rng.normal(s) * 0.05)(D, F) * (2.0 / D) ** 0.5),
            "w2": _w((lambda *s: _rng.normal(s) * 0.05)(F, D) * (2.0 / F) ** 0.5),
        }
    _B_in = _B_setup()

    return {
        "A_x": _A_in["x"],
        "A_wqkv": _A_in["wqkv"],
        "A_wo": _A_in["wo"],
        "B_x": _B_in["x"],
        "B_w1": _B_in["w1"],
        "B_w3": _B_in["w3"],
        "B_w2": _B_in["w2"],
    }

def reference(A_x, A_wqkv, A_wo, B_x, B_w1, B_w3, B_w2):
    def _A_ref(x, wqkv, wo):
        B, S, D = x.shape
        H = 32; Dh = D // H
        W, dil = 8, 2
        qkv = (lambda x, *d: x.transpose(*d))((x @ wqkv).reshape(B, S, 3, H, Dh), 2, 0, 3, 1, 4)
        q, k, v = qkv[0], qkv[1], qkv[2]
        scale = Dh ** -0.5
        pos = jnp.arange(S)
        off = jnp.arange(W) * dil
        idx = pos[:, None] - off[None, :]
        mask = idx >= 0
        idx_c = jnp.where(mask, idx, 0).reshape(-1)
        kg = k[:, :, idx_c, :].reshape(B, H, S, W, Dh)
        vg = v[:, :, idx_c, :].reshape(B, H, S, W, Dh)
        logits = jnp.einsum("bhsd,bhswd->bhsw", q, kg) * scale
        logits = jnp.where(mask[None, None, :, :], logits, -1e9)
        attn = _softmax(logits, axis=-1)
        o = jnp.einsum("bhsw,bhswd->bhsd", attn, vg)
        return (lambda x, *d: x.transpose(*d))(o, 0, 2, 1, 3).reshape(B, S, D) @ wo

    def _B_ref(x, w1, w3, w2):
        gate = jnp.einsum("bsd,df->bsf", x, w1)
        up = jnp.einsum("bsd,df->bsf", x, w3)
        h = _silu(gate) * up
        out = jnp.einsum("bsf,fd->bsd", h, w2)
        return out

    x = A_x
    xn = _layernorm(x, axis=-1)
    s = _A_ref(xn, A_wqkv, A_wo)
    g = _silu(_B_ref(xn, B_w1, B_w3, B_w2))
    return x + s * g
```

```python
import functools

import jax
import jax.numpy as jnp
from jax import lax
from jax.experimental import pallas as pl
from jax.experimental.pallas import tpu as pltpu

f32, bf16 = jnp.float32, jnp.bfloat16

S, D, F = 2048, 1024, 3584
H, DH, W, DIL = 32, 32, 8, 2
NT = D // 128
HALO = 16
PITCH = 33

_nn = functools.partial(jnp.dot, preferred_element_type=f32)


def _nt(a, b):
    return lax.dot_general(a, b, (((1,), (1,)), ((), ())), preferred_element_type=f32)


def _silu(x):
    hx = 0.5 * x
    return hx * (1.0 + jnp.tanh(hx))


def build(TM=256, FC=256, AR=32, LNR=64, G2=2, G3=2, flags=None):
    NP = TM // AR
    NC = F // FC
    NB = S // TM

    def kernel(xc_ref, xn_next_ref, wqkv_hbm, wo_hbm, w1_hbm, w3_hbm, w2_hbm, o_ref,
               wqkv_raw, wo_raw, w1s, w3s, w2s, wqkvp, wop, tsc,
               xn, qs, ks, vs, os_, hs, sem):
        i = pl.program_id(0)

        def cp_qkv(t):
            return pltpu.make_async_copy(wqkv_hbm.at[:, pl.ds(t * D, D)], wqkv_raw.at[t], sem.at[t])

        def cp_wo(n):
            return pltpu.make_async_copy(wo_hbm.at[:, pl.ds(n * 128, 128)], wo_raw.at[n], sem.at[4 + 2 * NC + NT + n])

        def cp_w1(c):
            return pltpu.make_async_copy(w1_hbm.at[:, pl.ds(c * FC, FC)], w1s.at[c], sem.at[4 + c])

        def cp_w3(c):
            return pltpu.make_async_copy(w3_hbm.at[:, pl.ds(c * FC, FC)], w3s.at[c], sem.at[4 + NC + c])

        def cp_w2(n):
            return pltpu.make_async_copy(w2_hbm.at[:, pl.ds(n * 128, 128)], w2s.at[n], sem.at[4 + 2 * NC + n])

        def layernorm(src_ref, r0, nr):
            x = src_ref[pl.ds(r0, nr), :].astype(f32)
            m = jnp.mean(x, axis=-1, keepdims=True)
            xc = x - m
            v = jnp.mean(xc * xc, axis=-1, keepdims=True)
            xn[pl.ds(r0, nr), :] = (xc * lax.rsqrt(v + 1e-5)).astype(bf16)

        def perm_cols(t, kt):
            k0 = pl.multiple_of(kt * 128, 128)
            for nt in range(NT):
                blk = wqkv_raw[t, pl.ds(k0, 128), pl.ds(nt * 128, 128)].astype(f32).T
                for hh in range(4):
                    tsc[kt, pl.ds(PITCH * (4 * nt + hh), 32), :] = blk[32 * hh:32 * hh + 32, :]
            for j in range(NT):
                for dlo in range(4):
                    wqkvp[t, kt, pl.ds(128 * j + 32 * dlo, 32), :] = (
                        tsc[kt, pl.ds(4 * j + dlo, 32, stride=PITCH), :].astype(bf16))

        def perm_wo(kt):
            for h in range(H):
                tsc[kt, pl.ds(PITCH * h, 32), :] = wo_raw[kt, pl.ds(32 * h, 32), :].astype(f32)
            for j in range(NT):
                for dlo in range(4):
                    wop[kt, pl.ds(128 * j + 32 * dlo, 32), :] = (
                        tsc[kt, pl.ds(4 * j + dlo, 32, stride=PITCH), :].astype(bf16))

        def qkv_tile(t, j):
            y = _nt(xn[...], jnp.concatenate([wqkvp[t, kt, pl.ds(j * 128, 128), :] for kt in range(NT)], axis=1))
            if t == 0:
                qs[j] = y * (DH ** -0.5)
            elif t == 1:
                ks[j, pl.ds(HALO, TM), :] = y
            else:
                vs[j, pl.ds(HALO, TM), :] = y

        def attention(p):
            r0 = p * AR
            q = [qs[j, pl.ds(r0, AR), :] for j in range(NT)]
            logits = []
            for w in range(W):
                acc = None
                for j in range(NT):
                    t_ = q[j] * ks[j, pl.ds(HALO + r0 - DIL * w, AR), :]
                    acc = t_ if acc is None else acc + t_
                acc = acc + pltpu.roll(acc, 64, 1)
                acc = acc + pltpu.roll(acc, 32, 1)
                if r0 < DIL * w:
                    row = i * TM + r0 + lax.broadcasted_iota(jnp.int32, (AR, 128), 0)
                    acc = jnp.where(row >= DIL * w, acc, -1e9)
                logits.append(acc)
            m = logits[0]
            for w in range(1, W):
                m = jnp.maximum(m, logits[w])
            e = [jnp.exp(l - m) for l in logits]
            den = e[0]
            for w in range(1, W):
                den = den + e[w]
            inv = 1.0 / den
            pr = [ew * inv for ew in e]
            for j in range(NT):
                acc = None
                for w in range(W):
                    t_ = pr[w] * vs[j, pl.ds(HALO + r0 - DIL * w, AR), :]
                    acc = t_ if acc is None else acc + t_
                os_[pl.ds(r0, AR), pl.ds(j * 128, 128)] = acc.astype(bf16)

        def gate_up(c):
            x_ = xn[...]
            g = _nn(x_, w1s[c])
            u = _nn(x_, w3s[c])
            hs[:, pl.ds(c * FC, FC)] = (_silu(g) * u).astype(bf16)

        def final_tile(n):
            ffn = _nn(hs[...], w2s[n])
            s = _nn(os_[...], wop[n])
            x_ = xc_ref[:, pl.ds(n * 128, 128)].astype(f32)
            o_ref[:, pl.ds(n * 128, 128)] = (x_ + s * _silu(ffn)).astype(o_ref.dtype)

        first = pl.when(i == 0)

        @first
        def _():
            cp_qkv(0).start(); cp_qkv(1).start(); cp_qkv(2).start()
            for c in range(NC):
                cp_w1(c).start(); cp_w3(c).start()
            for n in range(NT):
                cp_wo(n).start()
            for n in range(NT):
                cp_w2(n).start()
            for r in range(TM // LNR):
                layernorm(xc_ref, r * LNR, LNR)
            for j in range(NT):
                ks[j, pl.ds(TM, HALO), :] = jnp.zeros((HALO, 128), f32)
                vs[j, pl.ds(TM, HALO), :] = jnp.zeros((HALO, 128), f32)
            for t in range(3):
                cp_qkv(t).wait()
                @pl.loop(0, NT // 2)
                def _(kk):
                    perm_cols(t, 2 * kk)
                    perm_cols(t, 2 * kk + 1)

        for j in range(NT):
            ks[j, pl.ds(0, HALO), :] = ks[j, pl.ds(TM, HALO), :]
            vs[j, pl.ds(0, HALO), :] = vs[j, pl.ds(TM, HALO), :]
        for t in range(3):
            for j in range(NT):
                qkv_tile(t, j)
        for c in range(NC):
            if c % (NC // G2) == 0:
                @first
                def _():
                    for cc in range(c, c + NC // G2):
                        cp_w1(cc).wait(); cp_w3(cc).wait()
            gate_up(c)
            for p in range(NP):
                if (p * NC) // NP == c:
                    attention(p)
        nln = TM // LNR
        for n in range(NT):
            if n == 0:
                @first
                def _():
                    for nn in range(NT):
                        cp_wo(nn).wait()
                    @pl.loop(0, NT // 2)
                    def _(kk):
                        perm_wo(2 * kk)
                        perm_wo(2 * kk + 1)
            if n % (NT // G3) == 0:
                @first
                def _():
                    for nn in range(n, n + NT // G3):
                        cp_w2(nn).wait()
            final_tile(n)
            for r in range(nln):
                if (r * NT) // nln == n:
                    layernorm(xn_next_ref, r * LNR, LNR)

    nsem = 4 + 2 * NC + 2 * NT

    def run(x, wqkv, wo, w1, w3, w2):
        x2 = x.reshape(S, D)
        hbm = pl.BlockSpec(memory_space=pl.ANY)
        out = pl.pallas_call(
            kernel,
            grid=(NB,),
            in_specs=[
                pl.BlockSpec((TM, D), lambda i: (i, 0)),
                pl.BlockSpec((TM, D), lambda i: (jnp.minimum(i + 1, NB - 1), 0)),
                hbm, hbm, hbm, hbm, hbm,
            ],
            out_specs=pl.BlockSpec((TM, D), lambda i: (i, 0)),
            out_shape=jax.ShapeDtypeStruct((S, D), x.dtype),
            scratch_shapes=[
                pltpu.VMEM((3, D, D), bf16),
                pltpu.VMEM((NT, D, 128), bf16),
                pltpu.VMEM((NC, D, FC), bf16),
                pltpu.VMEM((NC, D, FC), bf16),
                pltpu.VMEM((NT, F, 128), bf16),
                pltpu.VMEM((3, NT, D, 128), bf16),
                pltpu.VMEM((NT, D, 128), bf16),
                pltpu.VMEM((NT, PITCH * H, 128), f32),
                pltpu.VMEM((TM, D), bf16),
                pltpu.VMEM((NT, TM, 128), f32),
                pltpu.VMEM((NT, HALO + TM, 128), f32),
                pltpu.VMEM((NT, HALO + TM, 128), f32),
                pltpu.VMEM((TM, D), bf16),
                pltpu.VMEM((TM, F), bf16),
                pltpu.SemaphoreType.DMA((nsem,)),
            ],
            compiler_params=pltpu.CompilerParams(
                dimension_semantics=("arbitrary",), vmem_limit_bytes=110 * 1024 * 1024, flags=flags),
        )(x2, x2, wqkv, wo, w1, w3, w2)
        return out.reshape(1, S, D)

    return run


@jax.jit
def pallas_recurrent_scan__sliding_local_dilated__glu_gated_swiglu__prompt_kernel(
    A_x, A_wqkv, A_wo, B_x, B_w1, B_w3, B_w2,
):
    del B_x
    return build()(A_x, A_wqkv, A_wo, B_w1, B_w3, B_w2)
```

```python
import functools

import jax
import jax.numpy as jnp
from jax import lax
from jax.experimental import pallas as pl
from jax.experimental.pallas import tpu as pltpu

f32, bf16 = jnp.float32, jnp.bfloat16

S, D, F = 2048, 1024, 3584
H, DH, W, DIL = 32, 32, 8, 2
NT = D // 128
HALO = 16
PITCH = 33

_nn = functools.partial(jnp.dot, preferred_element_type=f32)


def _nt(a, b):
    return lax.dot_general(a, b, (((1,), (1,)), ((), ())), preferred_element_type=f32)


def _silu(x):
    hx = 0.5 * x
    return hx * (1.0 + jnp.tanh(hx))


DEF_FLAGS = {"XLA_TPU_EVENLY_DISTRIBUTE_CRITICAL_NODES": True}


def build(TM=256, FC=256, AR=32, LNR=64, QM=256, flags=DEF_FLAGS, att_in="p2", order="gu"):
    NP = TM // AR
    NC = F // FC
    NB = S // TM
    NQ = S // QM
    KPI = NT // NQ

    def kernel(x_hbm, wqkv_hbm, wo_hbm, w1_hbm, w3_hbm, w2_hbm, o_ref,
               xs, xn, wqkv_raw, wo_raw, w1s, w3s, w2s, wqkvp, wop, tsc,
               qkv, os_, hs, sem):
        i = pl.program_id(0)

        def cp_x(rb):
            return pltpu.make_async_copy(x_hbm.at[pl.ds(rb * QM, QM), :], xs.at[pl.ds(rb * QM, QM), :], sem.at[rb])

        def cp_qkv(t):
            return pltpu.make_async_copy(wqkv_hbm.at[:, pl.ds(t * D, D)], wqkv_raw.at[t], sem.at[NQ + t])

        def cp_wo(n):
            return pltpu.make_async_copy(wo_hbm.at[:, pl.ds(n * 128, 128)], wo_raw.at[n], sem.at[NQ + 3 + n])

        cp_w1 = pltpu.make_async_copy(w1_hbm, w1s, sem.at[NQ + 3 + NT])
        cp_w3 = pltpu.make_async_copy(w3_hbm, w3s, sem.at[NQ + 4 + NT])
        cp_w2 = pltpu.make_async_copy(w2_hbm, w2s, sem.at[NQ + 5 + NT])

        def layernorm(r0, nr):
            x = xs[pl.ds(r0, nr), :].astype(f32)
            m = jnp.mean(x, axis=-1, keepdims=True)
            xc = x - m
            v = jnp.mean(xc * xc, axis=-1, keepdims=True)
            xn[pl.ds(r0, nr), :] = (xc * lax.rsqrt(v + 1e-5)).astype(bf16)

        def perm_cols(t, kt, slot, td=None):
            td = t if td is None else td
            k0 = pl.multiple_of(kt * 128, 128)
            for nt in range(NT):
                blk = wqkv_raw[t, pl.ds(k0, 128), pl.ds(nt * 128, 128)].astype(f32).T
                for hh in range(4):
                    tsc[slot, pl.ds(PITCH * (4 * nt + hh), 32), :] = blk[32 * hh:32 * hh + 32, :]
            for j in range(NT):
                for dlo in range(4):
                    wqkvp[td, kt, pl.ds(128 * j + 32 * dlo, 32), :] = (
                        tsc[slot, pl.ds(4 * j + dlo, 32, stride=PITCH), :].astype(bf16))

        def perm_wo(kt, slot):
            for h in range(H):
                tsc[slot, pl.ds(PITCH * h, 32), :] = wo_raw[kt, pl.ds(32 * h, 32), :].astype(f32)
            for j in range(NT):
                for dlo in range(4):
                    wop[kt, pl.ds(128 * j + 32 * dlo, 32), :] = (
                        tsc[slot, pl.ds(4 * j + dlo, 32, stride=PITCH), :].astype(bf16))

        def attention(p):
            r0 = p * AR
            base = pl.multiple_of(i * TM, TM)
            q = [qkv[0, j, pl.ds(base + (HALO + r0), AR), :] for j in range(NT)]
            logits = []
            for w in range(W):
                acc = None
                for j in range(NT):
                    t_ = q[j] * qkv[1, j, pl.ds(base + (HALO + r0 - DIL * w), AR), :]
                    acc = t_ if acc is None else acc + t_
                acc = acc + pltpu.roll(acc, 64, 1)
                acc = acc + pltpu.roll(acc, 32, 1)
                acc = acc * (DH ** -0.5)
                if r0 < DIL * w:
                    row = i * TM + r0 + lax.broadcasted_iota(jnp.int32, (AR, 128), 0)
                    acc = jnp.where(row >= DIL * w, acc, -1e9)
                logits.append(acc)
            m = logits[0]
            for w in range(1, W):
                m = jnp.maximum(m, logits[w])
            e = [jnp.exp(l - m) for l in logits]
            den = e[0]
            for w in range(1, W):
                den = den + e[w]
            inv = 1.0 / den
            pr = [ew * inv for ew in e]
            for j in range(NT):
                acc = None
                for w in range(W):
                    t_ = pr[w] * qkv[2, j, pl.ds(base + (HALO + r0 - DIL * w), AR), :]
                    acc = t_ if acc is None else acc + t_
                os_[pl.ds(r0, AR), pl.ds(j * 128, 128)] = acc.astype(bf16)

        def gate_up(x_, c):
            g = _nn(x_, w1s[:, pl.ds(c * FC, FC)])
            u = _nn(x_, w3s[:, pl.ds(c * FC, FC)])
            hs[:, pl.ds(c * FC, FC)] = (_silu(g) * u).astype(bf16)

        def final_tile(n):
            base = pl.multiple_of(i * TM, TM)
            ffn = _nn(hs[...], w2s[:, pl.ds(n * 128, 128)])
            s = _nn(os_[...], wop[n])
            x_ = xs[pl.ds(base, TM), pl.ds(n * 128, 128)].astype(f32)
            o_ref[:, pl.ds(n * 128, 128)] = (x_ + s * _silu(ffn)).astype(o_ref.dtype)

        @pl.when(i == 0)
        def _():
            cp_x(0).start()
            cp_qkv(0).start()
            for rb in range(1, NQ):
                cp_x(rb).start()
                if rb == 1:
                    cp_qkv(1).start()
            cp_qkv(2).start()
            for n in range(NT):
                cp_wo(n).start()
            cp_w1.start(); cp_w3.start(); cp_w2.start()
            for t in range(3):
                for j in range(NT):
                    qkv[t, j, pl.ds(0, HALO), :] = jnp.zeros((HALO, 128), f32)
            cp_x(0).wait()
            for r in range(QM // LNR):
                layernorm(r * LNR, LNR)
            cp_qkv(0).wait()

            @pl.loop(0, NT // 2)
            def _(kk):
                perm_cols(0, 2 * kk, 0)
                perm_cols(0, 2 * kk + 1, 1)

            @pl.loop(0, 3 * NQ)
            def _(it):
                t = it // NQ
                rb = it % NQ

                @pl.when(it < NQ - 1)
                def _():
                    cp_x(it + 1).wait()

                @pl.when(jnp.logical_and(rb == 0, t < 2))
                def _():
                    cp_qkv(t + 1).wait()

                r0 = pl.multiple_of(rb * QM, QM)
                x_ = xn[pl.ds(r0, QM), :]
                rn = pl.multiple_of(((rb + 1) % NQ) * QM, QM)
                tn = jnp.minimum(t + 1, 2)
                nln = QM // LNR
                for j in range(NT):
                    wt = jnp.concatenate([wqkvp[t, kt, pl.ds(j * 128, 128), :] for kt in range(NT)], axis=1)
                    y = _nt(x_, wt)

                    qkv[t, j, pl.ds(r0 + HALO, QM), :] = y
                    for r in range(nln):
                        if (r * NT) // nln == j:
                            layernorm(rn + r * LNR, LNR)
                    for kk in range(KPI):
                        if (kk * NT) // KPI == j:
                            perm_cols(tn, rb * KPI + kk, kk % 2, td=t + 1)

            for n in range(NT):
                cp_wo(n).wait()

            @pl.loop(0, NT // 2)
            def _(kk):
                perm_wo(2 * kk, 0)
                perm_wo(2 * kk + 1, 1)

            cp_w1.wait(); cp_w3.wait(); cp_w2.wait()

        base = pl.multiple_of(i * TM, TM)
        x_ = xn[pl.ds(base, TM), :]
        for c in range(NC):
            gate_up(x_, c)
            if att_in == "p2":
                for p in range(NP):
                    if (p * NC) // NP == c:
                        attention(p)
        for n in range(NT):
            final_tile(n)

    nsem = NQ + 6 + NT

    def run(x, wqkv, wo, w1, w3, w2):
        x2 = x.reshape(S, D)
        hbm = pl.BlockSpec(memory_space=pl.ANY)
        out = pl.pallas_call(
            kernel,
            grid=(NB,),
            in_specs=[hbm] * 6,
            out_specs=pl.BlockSpec((TM, D), lambda i: (i, 0)),
            out_shape=jax.ShapeDtypeStruct((S, D), x.dtype),
            scratch_shapes=[
                pltpu.VMEM((S, D), bf16),
                pltpu.VMEM((S, D), bf16),
                pltpu.VMEM((3, D, D), bf16),
                pltpu.VMEM((NT, D, 128), bf16),
                pltpu.VMEM((D, F), bf16),
                pltpu.VMEM((D, F), bf16),
                pltpu.VMEM((F, D), bf16),
                pltpu.VMEM((4, NT, D, 128), bf16),
                pltpu.VMEM((NT, D, 128), bf16),
                pltpu.VMEM((2, PITCH * H, 128), f32),
                pltpu.VMEM((3, NT, HALO + S, 128), f32),
                pltpu.VMEM((TM, D), bf16),
                pltpu.VMEM((TM, F), bf16),
                pltpu.SemaphoreType.DMA((nsem,)),
            ],
            compiler_params=pltpu.CompilerParams(
                dimension_semantics=("arbitrary",), vmem_limit_bytes=110 * 1024 * 1024, flags=flags),
        )(x2, wqkv, wo, w1, w3, w2)
        return out.reshape(1, S, D)

    return run


@jax.jit
def pallas_recurrent_scan__sliding_local_dilated__glu_gated_swiglu__prompt_kernel(
    A_x, A_wqkv, A_wo, B_x, B_w1, B_w3, B_w2,
):
    del B_x
    return build()(A_x, A_wqkv, A_wo, B_w1, B_w3, B_w2)
```

```python
import functools, contextlib

import jax
import jax.numpy as jnp
from jax import lax
from jax.experimental import pallas as pl
from jax.experimental.pallas import tpu as pltpu

f32, bf16 = jnp.float32, jnp.bfloat16

S, D, F = 2048, 1024, 3584
H, DH, W, DIL = 32, 32, 8, 2
NT = D // 128
HALO = 16
PITCH = 33

_nn = functools.partial(jnp.dot, preferred_element_type=f32)


def _nt(a, b):
    return lax.dot_general(a, b, (((1,), (1,)), ((), ())), preferred_element_type=f32)


def _silu(x):
    hx = 0.5 * x
    return hx * (1.0 + jnp.tanh(hx))


DEF_FLAGS = {"XLA_TPU_EVENLY_DISTRIBUTE_CRITICAL_NODES": True}


def build(scopes=False, TM=256, FC=256, AR=32, LNR=64, QM=256, QM1=512, QM2=512, flags=DEF_FLAGS, att_in="p2", order="gu"):
    NP = TM // AR
    NC = F // FC
    NB = S // TM
    NQ = S // QM

    def kernel(x_hbm, wqkv_hbm, wo_hbm, w1_hbm, w3_hbm, w2_hbm, o_ref,
               xs, xn, wqkv_raw, wo_raw, w1s, w3s, w2s, wqkvp, wop, tsc,
               qkv, os_, hs, sem):
        i = pl.program_id(0)

        sc = (lambda n: jax.named_scope(n)) if scopes else (lambda n: contextlib.nullcontext())
        def cp_x(rb):
            r0 = pl.multiple_of(rb * QM, QM)
            return pltpu.make_async_copy(x_hbm.at[pl.ds(r0, QM), :], xs.at[pl.ds(r0, QM), :], sem.at[rb])

        def cp_qkv(t, kt):
            k0 = pl.multiple_of(kt * 128, 128)
            return pltpu.make_async_copy(wqkv_hbm.at[pl.ds(k0, 128), pl.ds(t * D, D)],
                                         wqkv_raw.at[t, pl.ds(k0, 128), :], sem.at[NQ + t * NT + kt])

        def cp_wo(n):
            return pltpu.make_async_copy(wo_hbm.at[:, pl.ds(pl.multiple_of(n * 128, 128), 128)], wo_raw.at[n],
                                         sem.at[NQ + 3 * NT + n])

        cp_w1 = pltpu.make_async_copy(w1_hbm, w1s, sem.at[NQ + 4 * NT])
        cp_w3 = pltpu.make_async_copy(w3_hbm, w3s, sem.at[NQ + 4 * NT + 1])
        cp_w2 = pltpu.make_async_copy(w2_hbm, w2s, sem.at[NQ + 4 * NT + 2])

        def layernorm(r0, nr):
            x = xs[pl.ds(r0, nr), :].astype(f32)
            m = jnp.mean(x, axis=-1, keepdims=True)
            xc = x - m
            v = jnp.mean(xc * xc, axis=-1, keepdims=True)
            xn[pl.ds(r0, nr), :] = (xc * lax.rsqrt(v + 1e-5)).astype(bf16)

        def perm_cols(t, kt, slot, td=None):
            td = t if td is None else td
            k0 = pl.multiple_of(kt * 128, 128)
            for nt in range(NT):
                blk = wqkv_raw[t, pl.ds(k0, 128), pl.ds(nt * 128, 128)].astype(f32).T
                for hh in range(4):
                    tsc[slot, pl.ds(PITCH * (4 * nt + hh), 32), :] = blk[32 * hh:32 * hh + 32, :]
            for j in range(NT):
                for dlo in range(4):
                    wqkvp[td, kt, pl.ds(128 * j + 32 * dlo, 32), :] = (
                        tsc[slot, pl.ds(4 * j + dlo, 32, stride=PITCH), :].astype(bf16))

        def perm_wo(kt, slot):
            for h in range(H):
                tsc[slot, pl.ds(PITCH * h, 32), :] = wo_raw[kt, pl.ds(32 * h, 32), :].astype(f32)
            for j in range(NT):
                for dlo in range(4):
                    wop[kt, pl.ds(128 * j + 32 * dlo, 32), :] = (
                        tsc[slot, pl.ds(4 * j + dlo, 32, stride=PITCH), :].astype(bf16))

        def attention(p):
            r0 = p * AR
            base = pl.multiple_of(i * TM, TM)
            q = [qkv[0, j, pl.ds(base + (HALO + r0), AR), :] for j in range(NT)]
            logits = []
            for w in range(W):
                acc = None
                for j in range(NT):
                    t_ = q[j] * qkv[1, j, pl.ds(base + (HALO + r0 - DIL * w), AR), :]
                    acc = t_ if acc is None else acc + t_
                acc = acc + pltpu.roll(acc, 64, 1)
                acc = acc + pltpu.roll(acc, 32, 1)
                acc = acc * (DH ** -0.5)
                if r0 < DIL * w:
                    row = i * TM + r0 + lax.broadcasted_iota(jnp.int32, (AR, 128), 0)
                    acc = jnp.where(row >= DIL * w, acc, -1e9)
                logits.append(acc)
            m = logits[0]
            for w in range(1, W):
                m = jnp.maximum(m, logits[w])
            e = [jnp.exp(l - m) for l in logits]
            den = e[0]
            for w in range(1, W):
                den = den + e[w]
            inv = 1.0 / den
            pr = [ew * inv for ew in e]
            for j in range(NT):
                acc = None
                for w in range(W):
                    t_ = pr[w] * qkv[2, j, pl.ds(base + (HALO + r0 - DIL * w), AR), :]
                    acc = t_ if acc is None else acc + t_
                os_[pl.ds(r0, AR), pl.ds(j * 128, 128)] = acc.astype(bf16)

        def gate_up(x_, c):
            g = _nn(x_, w1s[:, pl.ds(c * FC, FC)])
            u = _nn(x_, w3s[:, pl.ds(c * FC, FC)])
            hs[:, pl.ds(c * FC, FC)] = (_silu(g) * u).astype(bf16)

        def final_tile(n):
            base = pl.multiple_of(i * TM, TM)
            ffn = _nn(hs[...], w2s[:, pl.ds(n * 128, 128)])
            s = _nn(os_[...], wop[n])
            x_ = xs[pl.ds(base, TM), pl.ds(n * 128, 128)].astype(f32)
            o_ref[:, pl.ds(n * 128, 128)] = (x_ + s * _silu(ffn)).astype(o_ref.dtype)

        @pl.when(i == 0)
        def _():
            cp_x(0).start()
            for kt in range(NT):
                cp_qkv(0, kt).start()
            cp_x(1).start()
            cp_qkv(1, 0).start()
            for t in range(3):
                for j in range(NT):
                    qkv[t, j, pl.ds(0, HALO), :] = jnp.zeros((HALO, 128), f32)
            with sc("waitx0"):
                cp_x(0).wait()
            with sc("ln0"):
                for r in range(QM // LNR):
                    layernorm(r * LNR, LNR)
            with sc("permq"):
                @pl.loop(0, NT // 2)
                def _(kk):
                    cp_qkv(0, 2 * kk).wait()
                    cp_qkv(0, 2 * kk + 1).wait()
                    perm_cols(0, 2 * kk, 0)
                    perm_cols(0, 2 * kk + 1, 1)

            def qkv_block(t, r0, qm, bg):
                x_ = xn[pl.ds(r0, qm), :]
                for j in range(NT):
                    wt = jnp.concatenate([wqkvp[t, kt, pl.ds(j * 128, 128), :] for kt in range(NT)], axis=1)
                    qkv[t, j, pl.ds(r0 + HALO, qm), :] = _nt(x_, wt)
                    bg(j)

            assert NQ == NT

            @pl.loop(0, NQ)
            @(jax.named_scope("ph1q") if scopes else (lambda f: f))
            def _(rb):
                @pl.when(rb + 1 < NQ)
                def _():
                    cp_x(rb + 1).wait()
                    cp_qkv(1, rb + 1).start()

                @pl.when(rb + 2 < NQ)
                def _():
                    cp_x(rb + 2).start()

                @pl.when(rb == NQ - 2)
                def _():
                    for kt in range(NT):
                        cp_qkv(2, kt).start()
                    for kt in range(NT):
                        cp_wo(kt).start()
                    cp_w1.start(); cp_w3.start(); cp_w2.start()

                cp_qkv(1, rb).wait()
                rn = pl.multiple_of(((rb + 1) % NQ) * QM, QM)
                nln = QM // LNR

                def bg(j):
                    for r in range(nln):
                        if (r * NT) // nln == j:
                            layernorm(rn + r * LNR, LNR)
                    if j == NT // 2:
                        perm_cols(1, rb, 0)

                qkv_block(0, pl.multiple_of(rb * QM, QM), QM, bg)

            n1 = S // QM1
            kp1 = NT // n1

            @pl.loop(0, n1)
            @(jax.named_scope("ph1k") if scopes else (lambda f: f))
            def _(rb):
                for kk in range(kp1):
                    cp_qkv(2, rb * kp1 + kk).wait()

                def bg(j):
                    for kk in range(kp1):
                        if (kk * NT) // kp1 + (NT // kp1) // 2 == j:
                            perm_cols(2, rb * kp1 + kk, kk % 2)

                qkv_block(1, pl.multiple_of(rb * QM1, QM1), QM1, bg)

            n2 = S // QM2
            kp2 = NT // n2

            @pl.loop(0, n2)
            @(jax.named_scope("ph1v") if scopes else (lambda f: f))
            def _(rb):
                for kk in range(kp2):
                    cp_wo(rb * kp2 + kk).wait()

                def bg(j):
                    for kk in range(kp2):
                        if (kk * NT) // kp2 + (NT // kp2) // 2 == j:
                            perm_wo(rb * kp2 + kk, kk % 2)

                qkv_block(2, pl.multiple_of(rb * QM2, QM2), QM2, bg)

            with sc("waitw"):
                cp_w1.wait(); cp_w3.wait(); cp_w2.wait()

        with sc('ph2'):
          base = pl.multiple_of(i * TM, TM)
          x_ = xn[pl.ds(base, TM), :]
          for c in range(NC):
              gate_up(x_, c)
              if att_in == "p2":
                  for p in range(NP):
                      if (p * NC) // NP == c:
                          attention(p)
          for n in range(NT):
              final_tile(n)

    nsem = NQ + 4 * NT + 3

    def run(x, wqkv, wo, w1, w3, w2):
        x2 = x.reshape(S, D)
        hbm = pl.BlockSpec(memory_space=pl.ANY)
        out = pl.pallas_call(
            kernel,
            grid=(NB,),
            in_specs=[hbm] * 6,
            out_specs=pl.BlockSpec((TM, D), lambda i: (i, 0)),
            out_shape=jax.ShapeDtypeStruct((S, D), x.dtype),
            scratch_shapes=[
                pltpu.VMEM((S, D), bf16),
                pltpu.VMEM((S, D), bf16),
                pltpu.VMEM((3, D, D), bf16),
                pltpu.VMEM((NT, D, 128), bf16),
                pltpu.VMEM((D, F), bf16),
                pltpu.VMEM((D, F), bf16),
                pltpu.VMEM((F, D), bf16),
                pltpu.VMEM((3, NT, D, 128), bf16),
                pltpu.VMEM((NT, D, 128), bf16),
                pltpu.VMEM((2, PITCH * H, 128), f32),
                pltpu.VMEM((3, NT, HALO + S, 128), f32),
                pltpu.VMEM((TM, D), bf16),
                pltpu.VMEM((TM, F), bf16),
                pltpu.SemaphoreType.DMA((nsem,)),
            ],
            compiler_params=pltpu.CompilerParams(
                dimension_semantics=("arbitrary",), vmem_limit_bytes=110 * 1024 * 1024, flags=flags),
        )(x2, wqkv, wo, w1, w3, w2)
        return out.reshape(1, S, D)

    return run


@jax.jit
def pallas_recurrent_scan__sliding_local_dilated__glu_gated_swiglu__prompt_kernel(
    A_x, A_wqkv, A_wo, B_x, B_w1, B_w3, B_w2,
):
    del B_x
    return build()(A_x, A_wqkv, A_wo, B_w1, B_w3, B_w2)
```

```python
import functools, contextlib

import jax
import jax.numpy as jnp
from jax import lax
from jax.experimental import pallas as pl
from jax.experimental.pallas import tpu as pltpu

f32, bf16 = jnp.float32, jnp.bfloat16

S, D, F = 2048, 1024, 3584
H, DH, W, DIL = 32, 32, 8, 2
NT = D // 128
HALO = 16
PITCH = 33

_nn = functools.partial(jnp.dot, preferred_element_type=f32)


def _nt(a, b):
    return lax.dot_general(a, b, (((1,), (1,)), ((), ())), preferred_element_type=f32)


def _silu(x):
    hx = 0.5 * x
    return hx * (1.0 + jnp.tanh(hx))


DEF_FLAGS = {"XLA_TPU_EVENLY_DISTRIBUTE_CRITICAL_NODES": True}


def build(scopes=False, TM=256, FC=256, AR=32, LNR=64, QM=256, QM1=512, flags=DEF_FLAGS,
          att_lo=0, att_hi=None, NQD=4, QM2=512, dep=False, att_in='p2'):
    vstat = False
    NP = TM // AR
    NC = F // FC
    NB = S // TM
    NQ = S // QM
    assert NQ == NT

    def kernel(x_hbm, wqkv_hbm, wo_hbm, w1_hbm, w3_hbm, w2_hbm, o_ref,
               xs, xn, wq_raw, wk_raw, wv_raw, wo_raw, w1s, w3s, w2s, wqp, wkp, wvp, wop, tsc,
               qs, ks, vs, os_, hs, sem):
        i = pl.program_id(0)
        sc = (lambda n: jax.named_scope(n)) if scopes else (lambda n: contextlib.nullcontext())
        SEM_X0, SEM_G, SEM_V, SEM_W, SEM_Q = 0, 1, 4, 5, 6
        GROUPS = ((1, 1, 0, 1), (2, 2, 1, 2), (4, 4, 3, 5))

        def cp_x(r0, nr, s_):
            return pltpu.make_async_copy(x_hbm.at[pl.ds(r0, nr), :], xs.at[pl.ds(r0, nr), :], sem.at[s_])

        def cp_q(c):
            n = D // NQD
            k0 = pl.multiple_of(c * n, n)
            return pltpu.make_async_copy(wqkv_hbm.at[pl.ds(k0, n), pl.ds(0, D)], wq_raw.at[pl.ds(k0, n), :],
                                         sem.at[SEM_Q + c])

        def cp_k(k0, nk, s_):
            return pltpu.make_async_copy(wqkv_hbm.at[pl.ds(k0, nk), pl.ds(D, D)], wk_raw.at[pl.ds(k0, nk), :],
                                         sem.at[s_])

        def cp_group(g):
            xb, xnb, kb, knb = GROUPS[g]
            return (cp_x(xb * QM, xnb * QM, SEM_G + g), cp_k(kb * 128, knb * 128, SEM_G + g))

        cp_v = pltpu.make_async_copy(wqkv_hbm.at[:, pl.ds(2 * D, D)], wv_raw, sem.at[SEM_V])

        def cp_wo(n):
            return pltpu.make_async_copy(wo_hbm.at[:, pl.ds(n * 128, 128)], wo_raw.at[n], sem.at[SEM_V])

        cp_w1 = pltpu.make_async_copy(w1_hbm, w1s, sem.at[SEM_W])
        cp_w3 = pltpu.make_async_copy(w3_hbm, w3s, sem.at[SEM_W])
        cp_w2 = pltpu.make_async_copy(w2_hbm, w2s, sem.at[SEM_W])

        def layernorm(r0, nr):
            x = xs[pl.ds(r0, nr), :].astype(f32)
            m = jnp.mean(x, axis=-1, keepdims=True)
            xc = x - m
            v = jnp.mean(xc * xc, axis=-1, keepdims=True)
            xn[pl.ds(r0, nr), :] = (xc * lax.rsqrt(v + 1e-5)).astype(bf16)

        def perm_cols(src, dst, kt, slot):
            k0 = pl.multiple_of(kt * 128, 128)
            for nt in range(NT):
                blk = src[pl.ds(k0, 128), pl.ds(nt * 128, 128)].astype(f32).T
                for hh in range(4):
                    tsc[slot, pl.ds(PITCH * (4 * nt + hh), 32), :] = blk[32 * hh:32 * hh + 32, :]
            for j in range(NT):
                for dlo in range(4):
                    dst[kt, pl.ds(128 * j + 32 * dlo, 32), :] = (
                        tsc[slot, pl.ds(4 * j + dlo, 32, stride=PITCH), :].astype(bf16))

        def perm_wo(kt, slot):
            for h in range(H):
                tsc[slot, pl.ds(PITCH * h, 32), :] = wo_raw[kt, pl.ds(32 * h, 32), :].astype(f32)
            for j in range(NT):
                for dlo in range(4):
                    wop[kt, pl.ds(128 * j + 32 * dlo, 32), :] = (
                        tsc[slot, pl.ds(4 * j + dlo, 32, stride=PITCH), :].astype(bf16))

        def proj_block(wp, dst, r0, qm, bg, d0=None):
            d0 = r0 if d0 is None else d0
            x_ = xn[pl.ds(r0, qm), :]
            for j in range(NT):
                wt = jnp.concatenate([wp[kt, pl.ds(j * 128, 128), :] for kt in range(NT)], axis=1)
                dst[j, pl.ds(d0 + HALO, qm), :] = _nt(x_, wt)
                bg(j)

        def attention(p, dv=None):
            r0 = p * AR
            base = pl.multiple_of(i * TM, TM)
            q = [qs[j, pl.ds(base + (HALO + r0), AR), :] for j in range(NT)]
            if dv is not None:
                q = [jnp.where(i < 0, dv, qj) for qj in q]
            logits = []
            for w in range(W):
                acc = None
                for j in range(NT):
                    t_ = q[j] * ks[j, pl.ds(base + (HALO + r0 - DIL * w), AR), :]
                    acc = t_ if acc is None else acc + t_
                acc = acc + pltpu.roll(acc, 64, 1)
                acc = acc + pltpu.roll(acc, 32, 1)
                acc = acc * (DH ** -0.5)
                if r0 < DIL * w:
                    row = i * TM + r0 + lax.broadcasted_iota(jnp.int32, (AR, 128), 0)
                    acc = jnp.where(row >= DIL * w, acc, -1e9)
                logits.append(acc)
            m = logits[0]
            for w in range(1, W):
                m = jnp.maximum(m, logits[w])
            e = [jnp.exp(l - m) for l in logits]
            den = e[0]
            for w in range(1, W):
                den = den + e[w]
            inv = 1.0 / den
            pr = [ew * inv for ew in e]
            for j in range(NT):
                acc = None
                for w in range(W):
                    vb = 0 if vstat else base
                    t_ = pr[w] * vs[j, pl.ds(vb + (HALO + r0 - DIL * w), AR), :]
                    acc = t_ if acc is None else acc + t_
                os_[pl.ds(r0, AR), pl.ds(j * 128, 128)] = acc.astype(bf16)

        def gate_up(x_, c):
            g = _nn(x_, w1s[:, pl.ds(c * FC, FC)])
            u = _nn(x_, w3s[:, pl.ds(c * FC, FC)])
            hv = _silu(g) * u
            hs[:, pl.ds(c * FC, FC)] = hv.astype(bf16)
            return hv[:AR, :128]

        def final_tile(n):
            base = pl.multiple_of(i * TM, TM)
            ffn = _nn(hs[...], w2s[:, pl.ds(n * 128, 128)])
            s = _nn(os_[...], wop[n])
            x_ = xs[pl.ds(base, TM), pl.ds(n * 128, 128)].astype(f32)
            o_ref[:, pl.ds(n * 128, 128)] = (x_ + s * _silu(ffn)).astype(o_ref.dtype)

        @pl.when(i == 0)
        def _():
            cp_x(0, QM, SEM_X0).start()
            for c in range(NQD):
                cp_q(c).start()
            for g in range(3):
                for cp in cp_group(g):
                    cp.start()
            cp_v.start()
            for kt in range(NT):
                cp_wo(kt).start()
            cp_w1.start(); cp_w3.start(); cp_w2.start()
            for j in range(NT):
                ks[j, pl.ds(0, HALO), :] = jnp.zeros((HALO, 128), f32)
                vs[j, pl.ds(TM if vstat else 0, HALO), :] = jnp.zeros((HALO, 128), f32)
            with sc("waitx0"):
                cp_x(0, QM, SEM_X0).wait()
            with sc("ln0"):
                for r in range(QM // LNR):
                    layernorm(r * LNR, LNR)
            with sc("permq"):
                cpk = NT // NQD
                for c in range(NQD):
                    cp_q(c).wait()
                    for kk in range(cpk):
                        perm_cols(wq_raw, wqp, c * cpk + kk, kk % 2)

            @pl.loop(0, NQ)
            @(jax.named_scope("ph1q") if scopes else (lambda f: f))
            def _(rb):
                for g, at in enumerate((0, 1, 3)):
                    @pl.when(rb == at)
                    def _():
                        for cp in cp_group(g):
                            cp.wait()

                rn = pl.multiple_of(((rb + 1) % NQ) * QM, QM)
                nln = QM // LNR

                def bg(j):
                    for r in range(nln):
                        if (r * NT) // nln == j:
                            layernorm(rn + r * LNR, LNR)
                    if j == NT // 2:
                        perm_cols(wk_raw, wkp, rb, 0)

                proj_block(wqp, qs, pl.multiple_of(rb * QM, QM), QM, bg)

            cp_v.wait()
            for kt in range(NT):
                cp_wo(kt).wait()
            n1 = S // QM1
            kp1 = NT // n1

            @pl.loop(0, n1)
            @(jax.named_scope("ph1k") if scopes else (lambda f: f))
            def _(rb):
                def bg(j):
                    for kk in range(kp1):
                        if (kk * NT) // kp1 + (NT // kp1) // 2 == j:
                            perm_cols(wv_raw, wvp, rb * kp1 + kk, kk % 2)

                proj_block(wkp, ks, pl.multiple_of(rb * QM1, QM1), QM1, bg)

            n2 = S // QM2
            kp2 = NT // n2

            @pl.loop(0, n2)
            @(jax.named_scope("ph1v") if scopes else (lambda f: f))
            def _(rb):
                def bg(j):
                    for kk in range(kp2):
                        if (kk * NT) // kp2 + (NT // kp2) // 2 == j:
                            perm_wo(rb * kp2 + kk, kk % 2)

                proj_block(wvp, vs, pl.multiple_of(rb * QM2, QM2), QM2, bg)

            with sc("waitw"):
                cp_w1.wait(); cp_w3.wait(); cp_w2.wait()

        with sc('ph2'):
            base = pl.multiple_of(i * TM, TM)
            x_ = xn[pl.ds(base, TM), :]
            hi = NC if att_hi is None else att_hi
            dv = None
            for c in range(NC):
                for p in range(NP):
                    if att_lo + (p * (hi - att_lo)) // NP == c:
                        attention(p, dv if dep else None)
                dv = gate_up(x_, c)
            for n in range(NT):
                final_tile(n)

    nsem = 6 + NQD

    def run(x, wqkv, wo, w1, w3, w2):
        x2 = x.reshape(S, D)
        hbm = pl.BlockSpec(memory_space=pl.ANY)
        wp = lambda: pltpu.VMEM((NT, D, 128), bf16)
        out = pl.pallas_call(
            kernel,
            grid=(NB,),
            in_specs=[hbm] * 6,
            out_specs=pl.BlockSpec((TM, D), lambda i: (i, 0)),
            out_shape=jax.ShapeDtypeStruct((S, D), x.dtype),
            scratch_shapes=[
                pltpu.VMEM((S, D), bf16),
                pltpu.VMEM((S, D), bf16),
                pltpu.VMEM((D, D), bf16),
                pltpu.VMEM((D, D), bf16),
                pltpu.VMEM((D, D), bf16),
                wp(),
                pltpu.VMEM((D, F), bf16),
                pltpu.VMEM((D, F), bf16),
                pltpu.VMEM((F, D), bf16),
                wp(), wp(), wp(), wp(),
                pltpu.VMEM((2, PITCH * H, 128), f32),
                pltpu.VMEM((NT, HALO + S, 128), f32),
                pltpu.VMEM((NT, HALO + S, 128), f32),
                pltpu.VMEM((NT, HALO + (TM if vstat else S), 128), f32),
                pltpu.VMEM((TM, D), bf16),
                pltpu.VMEM((TM, F), bf16),
                pltpu.SemaphoreType.DMA((nsem,)),
            ],
            compiler_params=pltpu.CompilerParams(
                dimension_semantics=("arbitrary",), vmem_limit_bytes=110 * 1024 * 1024, flags=flags),
        )(x2, wqkv, wo, w1, w3, w2)
        return out.reshape(1, S, D)

    return run


@jax.jit
def pallas_recurrent_scan__sliding_local_dilated__glu_gated_swiglu__prompt_kernel(
    A_x, A_wqkv, A_wo, B_x, B_w1, B_w3, B_w2,
):
    del B_x
    return build()(A_x, A_wqkv, A_wo, B_w1, B_w3, B_w2)
```

```python
import functools, contextlib

import jax
import jax.numpy as jnp
from jax import lax
from jax.experimental import pallas as pl
from jax.experimental.pallas import tpu as pltpu

f32, bf16 = jnp.float32, jnp.bfloat16

S, D, F = 2048, 1024, 3584
H, DH, W, DIL = 32, 32, 8, 2
NT = D // 128
HALO = 16
PITCH = 33

_nn = functools.partial(jnp.dot, preferred_element_type=f32)


def _nt(a, b):
    return lax.dot_general(a, b, (((1,), (1,)), ((), ())), preferred_element_type=f32)


def _silu(x):
    hx = 0.5 * x
    return hx * (1.0 + jnp.tanh(hx))


DEF_FLAGS = {"XLA_TPU_EVENLY_DISTRIBUTE_CRITICAL_NODES": True}


def build(scopes=False, TM=256, FC=128, AR=8, LNR=64, QM=256, QM1=512, flags=DEF_FLAGS,
          att_lo=1, att_hi=27, NQD=4, QM2=512, dep=True, att_in='p2', osplit=5, kvm=False):
    vstat = False
    NP = TM // AR
    NC = F // FC
    NB = S // TM
    NQ = S // QM
    assert NQ == NT

    def kernel(x_hbm, wqkv_hbm, wo_hbm, w1_hbm, w3_hbm, w2_hbm, o_ref,
               xs, xn, wq_raw, wk_raw, wv_raw, wo_raw, w1s, w3s, w2s, wqp, wkp, wvp, wop, tsc,
               qs, ks, vs, os_, hs, ost, gs, sem):
        i = pl.program_id(0)
        sc = (lambda n: jax.named_scope(n)) if scopes else (lambda n: contextlib.nullcontext())
        SEM_X0, SEM_G, SEM_V, SEM_W, SEM_O, SEM_Q = 0, 1, 4, 5, 6, 8
        GROUPS = ((1, 1, 0, 1), (2, 2, 1, 2), (4, 4, 3, 5))

        def cp_x(r0, nr, s_):
            return pltpu.make_async_copy(x_hbm.at[pl.ds(r0, nr), :], xs.at[pl.ds(r0, nr), :], sem.at[s_])

        def cp_q(c):
            n = D // NQD
            k0 = pl.multiple_of(c * n, n)
            return pltpu.make_async_copy(wqkv_hbm.at[pl.ds(k0, n), pl.ds(0, D)], wq_raw.at[pl.ds(k0, n), :],
                                         sem.at[SEM_Q + c])

        def cp_k(k0, nk, s_):
            return pltpu.make_async_copy(wqkv_hbm.at[pl.ds(k0, nk), pl.ds(D, D)], wk_raw.at[pl.ds(k0, nk), :],
                                         sem.at[s_])

        def cp_group(g):
            xb, xnb, kb, knb = GROUPS[g]
            return (cp_x(xb * QM, xnb * QM, SEM_G + g), cp_k(kb * 128, knb * 128, SEM_G + g))

        def cp_o(step, part):
            c0, nc = ((0, (osplit + 1) * 128), ((osplit + 1) * 128, D - (osplit + 1) * 128))[part]
            r0 = pl.multiple_of(step * TM, TM)
            return pltpu.make_async_copy(ost.at[step % 2, :, pl.ds(c0, nc)], o_ref.at[pl.ds(r0, TM), pl.ds(c0, nc)], sem.at[SEM_O + step % 2])

        cp_v = pltpu.make_async_copy(wqkv_hbm.at[:, pl.ds(2 * D, D)], wv_raw, sem.at[SEM_V])

        def cp_wo(n):
            return pltpu.make_async_copy(wo_hbm.at[:, pl.ds(n * 128, 128)], wo_raw.at[n], sem.at[SEM_V])

        cp_w1 = pltpu.make_async_copy(w1_hbm, w1s, sem.at[SEM_W])
        cp_w3 = pltpu.make_async_copy(w3_hbm, w3s, sem.at[SEM_W])
        cp_w2 = pltpu.make_async_copy(w2_hbm, w2s, sem.at[SEM_W])

        def layernorm(r0, nr):
            x = xs[pl.ds(r0, nr), :].astype(f32)
            m = jnp.mean(x, axis=-1, keepdims=True)
            xc = x - m
            v = jnp.mean(xc * xc, axis=-1, keepdims=True)
            xn[pl.ds(r0, nr), :] = (xc * lax.rsqrt(v + 1e-5)).astype(bf16)

        def perm_cols(src, dst, kt, slot):
            k0 = pl.multiple_of(kt * 128, 128)
            for nt in range(NT):
                blk = src[pl.ds(k0, 128), pl.ds(nt * 128, 128)].astype(f32).T
                for hh in range(4):
                    tsc[slot, pl.ds(PITCH * (4 * nt + hh), 32), :] = blk[32 * hh:32 * hh + 32, :]
            for j in range(NT):
                for dlo in range(4):
                    dst[kt, pl.ds(128 * j + 32 * dlo, 32), :] = (
                        tsc[slot, pl.ds(4 * j + dlo, 32, stride=PITCH), :].astype(bf16))

        def perm_wo(kt, slot):
            for h in range(H):
                tsc[slot, pl.ds(PITCH * h, 32), :] = wo_raw[kt, pl.ds(32 * h, 32), :].astype(f32)
            for j in range(NT):
                for dlo in range(4):
                    wop[kt, pl.ds(128 * j + 32 * dlo, 32), :] = (
                        tsc[slot, pl.ds(4 * j + dlo, 32, stride=PITCH), :].astype(bf16))

        def proj_block(wp, dst, r0, qm, bg, d0=None):
            d0 = r0 if d0 is None else d0
            x_ = xn[pl.ds(r0, qm), :]
            for j in range(NT):
                wt = jnp.concatenate([wp[kt, pl.ds(j * 128, 128), :] for kt in range(NT)], axis=1)
                dst[j, pl.ds(d0 + HALO, qm), :] = _nt(x_, wt)
                bg(j)

        def attention(p, dv=None):
            r0 = p * AR
            base = pl.multiple_of(i * TM, TM)
            q = [qs[j, pl.ds(base + (HALO + r0), AR), :] for j in range(NT)]
            if dv is not None:
                q = [jnp.where(i < 0, dv, qj) for qj in q]
            logits = []
            for w in range(W):
                acc = None
                for j in range(NT):
                    t_ = q[j] * ks[j, pl.ds(base + (HALO + r0 - DIL * w), AR), :]
                    acc = t_ if acc is None else acc + t_
                acc = acc + pltpu.roll(acc, 64, 1)
                acc = acc + pltpu.roll(acc, 32, 1)
                acc = acc * (DH ** -0.5)
                if r0 < DIL * w:
                    row = i * TM + r0 + lax.broadcasted_iota(jnp.int32, (AR, 128), 0)
                    acc = jnp.where(row >= DIL * w, acc, -1e9)
                logits.append(acc)
            m = logits[0]
            for w in range(1, W):
                m = jnp.maximum(m, logits[w])
            e = [jnp.exp(l - m) for l in logits]
            den = e[0]
            for w in range(1, W):
                den = den + e[w]
            inv = 1.0 / den
            pr = [ew * inv for ew in e]
            for j in range(NT):
                acc = None
                for w in range(W):
                    vb = 0 if vstat else base
                    t_ = pr[w] * vs[j, pl.ds(vb + (HALO + r0 - DIL * w), AR), :]
                    acc = t_ if acc is None else acc + t_
                os_[pl.ds(r0, AR), pl.ds(j * 128, 128)] = acc.astype(bf16)

        def gate_up(x_, c):
            g = _nn(x_, w1s[:, pl.ds(c * FC, FC)])
            u = _nn(x_, w3s[:, pl.ds(c * FC, FC)])
            hv = _silu(g) * u
            hs[:, pl.ds(c * FC, FC)] = hv.astype(bf16)
            return hv[:AR, :128]

        def final_tile(n):
            base = pl.multiple_of(i * TM, TM)
            ffn = _nn(hs[...], w2s[:, pl.ds(n * 128, 128)])
            s = _nn(os_[...], wop[n])
            x_ = xs[pl.ds(base, TM), pl.ds(n * 128, 128)].astype(f32)
            ost[i % 2, :, pl.ds(n * 128, 128)] = (x_ + s * _silu(ffn)).astype(ost.dtype)

        @pl.when(i == 0)
        def _():
            cp_x(0, QM, SEM_X0).start()
            for c in range(NQD):
                cp_q(c).start()
            for g in range(3):
                for cp in cp_group(g):
                    cp.start()
            cp_v.start()
            for kt in range(NT):
                cp_wo(kt).start()
            cp_w1.start(); cp_w3.start(); cp_w2.start()
            for j in range(NT):
                ks[j, pl.ds(0, HALO), :] = jnp.zeros((HALO, 128), f32)
                vs[j, pl.ds(TM if vstat else 0, HALO), :] = jnp.zeros((HALO, 128), f32)
            with sc("waitx0"):
                cp_x(0, QM, SEM_X0).wait()
            with sc("ln0"):
                for r in range(QM // LNR):
                    layernorm(r * LNR, LNR)
            with sc("permq"):
                cpk = NT // NQD

                @pl.loop(0, NQD)
                def _(c):
                    cp_q(c).wait()
                    for kk in range(cpk):
                        perm_cols(wq_raw, wqp, c * cpk + kk, kk % 2)

            @pl.loop(0, NQ)
            @(jax.named_scope("ph1q") if scopes else (lambda f: f))
            def _(rb):
                for g, at in enumerate((0, 1, 3)):
                    @pl.when(rb == at)
                    def _():
                        for cp in cp_group(g):
                            cp.wait()

                rn = pl.multiple_of(((rb + 1) % NQ) * QM, QM)
                nln = QM // LNR

                def bg(j):
                    for r in range(nln):
                        if (r * NT) // nln == j:
                            layernorm(rn + r * LNR, LNR)
                    if j == NT // 2:
                        perm_cols(wk_raw, wkp, rb, 0)

                proj_block(wqp, qs, pl.multiple_of(rb * QM, QM), QM, bg)

            cp_v.wait()
            for kt in range(NT):
                cp_wo(kt).wait()
            if kvm:
                n1 = S // QM1
                kp1 = NT // n1

                @pl.loop(0, n1)
                @(jax.named_scope("ph1kv") if scopes else (lambda f: f))
                def _(rb):
                    r0 = pl.multiple_of(rb * QM1, QM1)
                    proj_block(wkp, ks, r0, QM1, lambda j: perm_cols(wv_raw, wvp, j, j % 2))

                    def bg(j):
                        for kk in range(kp1):
                            if (kk * NT) // kp1 + (NT // kp1) // 2 == j:
                                perm_wo(rb * kp1 + kk, kk % 2)

                    proj_block(wvp, vs, r0, QM1, bg)
            else:
                n1 = S // QM1
                kp1 = NT // n1

                @pl.loop(0, n1)
                @(jax.named_scope("ph1k") if scopes else (lambda f: f))
                def _(rb):
                    def bg(j):
                        for kk in range(kp1):
                            if (kk * NT) // kp1 + (NT // kp1) // 2 == j:
                                perm_cols(wv_raw, wvp, rb * kp1 + kk, kk % 2)

                    proj_block(wkp, ks, pl.multiple_of(rb * QM1, QM1), QM1, bg)

                n2 = S // QM2
                kp2 = NT // n2

                @pl.loop(0, n2)
                @(jax.named_scope("ph1v") if scopes else (lambda f: f))
                def _(rb):
                    def bg(j):
                        for kk in range(kp2):
                            if (kk * NT) // kp2 + (NT // kp2) // 2 == j:
                                perm_wo(rb * kp2 + kk, kk % 2)

                    proj_block(wvp, vs, pl.multiple_of(rb * QM2, QM2), QM2, bg)

            with sc("waitw"):
                cp_w1.wait(); cp_w3.wait(); cp_w2.wait()

        @pl.when(i > 1)
        def _():
            cp_o(i - 2, 0).wait()
            cp_o(i - 2, 1).wait()

        with sc('ph2'):
            base = pl.multiple_of(i * TM, TM)
            x_ = xn[pl.ds(base, TM), :]
            if att_in == 'p2':
                hi = NC if att_hi is None else att_hi
                dv = None
                for c in range(NC):
                    for p in range(NP):
                        if att_lo + (p * (hi - att_lo)) // NP == c:
                            attention(p, dv if dep else None)
                    dv = gate_up(x_, c)
                for n in range(NT):
                    final_tile(n)
                    if n == osplit:
                        cp_o(i, 0).start()
            else:
                dv = None
                for c in range(NC):
                    dv = gate_up(x_, c)
                hi = NT if att_hi is None else att_hi
                for n in range(NT):
                    for p in range(NP):
                        if att_lo + (p * (hi - att_lo)) // NP == n:
                            attention(p, dv if dep else None)
                    g = _silu(_nn(hs[...], w2s[:, pl.ds(n * 128, 128)]))
                    gs[:, pl.ds(n * 128, 128)] = g
                    dv = g[:AR, :]
                for n in range(NT):
                    s_ = _nn(os_[...], wop[n])
                    xr = xs[pl.ds(base, TM), pl.ds(n * 128, 128)].astype(f32)
                    ost[i % 2, :, pl.ds(n * 128, 128)] = (xr + s_ * gs[:, pl.ds(n * 128, 128)]).astype(ost.dtype)
                    if n == osplit:
                        cp_o(i, 0).start()
            cp_o(i, 1).start()

        @pl.when(i == NB - 1)
        def _():
            cp_o(i - 1, 0).wait()
            cp_o(i - 1, 1).wait()
            cp_o(i, 0).wait()
            cp_o(i, 1).wait()

    nsem = 8 + NQD

    def run(x, wqkv, wo, w1, w3, w2):
        x2 = x.reshape(S, D)
        hbm = pl.BlockSpec(memory_space=pl.ANY)
        wp = lambda: pltpu.VMEM((NT, D, 128), bf16)
        out = pl.pallas_call(
            kernel,
            grid=(NB,),
            in_specs=[hbm] * 6,
            out_specs=hbm,
            out_shape=jax.ShapeDtypeStruct((S, D), x.dtype),
            scratch_shapes=[
                pltpu.VMEM((S, D), bf16),
                pltpu.VMEM((S, D), bf16),
                pltpu.VMEM((D, D), bf16),
                pltpu.VMEM((D, D), bf16),
                pltpu.VMEM((D, D), bf16),
                wp(),
                pltpu.VMEM((D, F), bf16),
                pltpu.VMEM((D, F), bf16),
                pltpu.VMEM((F, D), bf16),
                wp(), wp(), wp(), wp(),
                pltpu.VMEM((2, PITCH * H, 128), f32),
                pltpu.VMEM((NT, HALO + S, 128), f32),
                pltpu.VMEM((NT, HALO + S, 128), f32),
                pltpu.VMEM((NT, HALO + (TM if vstat else S), 128), f32),
                pltpu.VMEM((TM, D), bf16),
                pltpu.VMEM((TM, F), bf16),
                pltpu.VMEM((2, TM, D), bf16),
                pltpu.VMEM((TM, D), f32),
                pltpu.SemaphoreType.DMA((nsem,)),
            ],
            compiler_params=pltpu.CompilerParams(
                dimension_semantics=("arbitrary",), vmem_limit_bytes=110 * 1024 * 1024, flags=flags),
        )(x2, wqkv, wo, w1, w3, w2)
        return out.reshape(1, S, D)

    return run


@jax.jit
def pallas_recurrent_scan__sliding_local_dilated__glu_gated_swiglu__prompt_kernel(
    A_x, A_wqkv, A_wo, B_x, B_w1, B_w3, B_w2,
):
    del B_x
    return build()(A_x, A_wqkv, A_wo, B_w1, B_w3, B_w2)
```

```python
import functools, contextlib

import jax
import jax.numpy as jnp
from jax import lax
from jax.experimental import pallas as pl
from jax.experimental.pallas import tpu as pltpu

f32, bf16 = jnp.float32, jnp.bfloat16

S, D, F = 2048, 1024, 3584
H, DH, W, DIL = 32, 32, 8, 2
NT = D // 128
HALO = 16
PITCH = 33

_nn = functools.partial(jnp.dot, preferred_element_type=f32)


def _nt(a, b):
    return lax.dot_general(a, b, (((1,), (1,)), ((), ())), preferred_element_type=f32)


def _silu(x):
    hx = 0.5 * x
    return hx * (1.0 + jnp.tanh(hx))


DEF_FLAGS = {"XLA_TPU_EVENLY_DISTRIBUTE_CRITICAL_NODES": True}


def build(scopes=False, TM=256, FC=128, AR=8, LNR=64, QM=256, QM1=512, flags=DEF_FLAGS,
          att_lo=1, att_hi=27, NQD=4, QM2=512, dep=True, att_in='p2', osplit=5, kvm=True, pdep=True, wa=0, wb=2, vdep=True, kdep=False, qdep=False):
    vstat = False
    NP = TM // AR
    NC = F // FC
    NB = S // TM
    NQ = S // QM
    assert NQ == NT

    def kernel(x_hbm, wqkv_hbm, wo_hbm, w1_hbm, w3_hbm, w2_hbm, o_ref,
               xs, xn, wq_raw, wk_raw, wv_raw, wo_raw, w1s, w3s, w2s, wqp, wkp, wvp, wop, tsc,
               qs, ks, vs, os_, hs, ost, gs, sem):
        i = pl.program_id(0)
        sc = (lambda n: jax.named_scope(n)) if scopes else (lambda n: contextlib.nullcontext())
        SEM_X0, SEM_G, SEM_V, SEM_W, SEM_O, SEM_Q = 0, 1, 4, 5, 6, 8
        GROUPS = ((1, 1, 0, 1), (2, 2, 1, 2), (4, 4, 3, 5))

        def cp_x(r0, nr, s_):
            return pltpu.make_async_copy(x_hbm.at[pl.ds(r0, nr), :], xs.at[pl.ds(r0, nr), :], sem.at[s_])

        def cp_q(c):
            n = D // NQD
            k0 = pl.multiple_of(c * n, n)
            return pltpu.make_async_copy(wqkv_hbm.at[pl.ds(k0, n), pl.ds(0, D)], wq_raw.at[pl.ds(k0, n), :],
                                         sem.at[SEM_Q + c])

        def cp_k(k0, nk, s_):
            return pltpu.make_async_copy(wqkv_hbm.at[pl.ds(k0, nk), pl.ds(D, D)], wk_raw.at[pl.ds(k0, nk), :],
                                         sem.at[s_])

        def cp_group(g):
            xb, xnb, kb, knb = GROUPS[g]
            return (cp_x(xb * QM, xnb * QM, SEM_G + g), cp_k(kb * 128, knb * 128, SEM_G + g))

        def cp_o(step, part):
            c0, nc = ((0, (osplit + 1) * 128), ((osplit + 1) * 128, D - (osplit + 1) * 128))[part]
            r0 = pl.multiple_of(step * TM, TM)
            return pltpu.make_async_copy(ost.at[step % 2, :, pl.ds(c0, nc)], o_ref.at[pl.ds(r0, TM), pl.ds(c0, nc)], sem.at[SEM_O + step % 2])

        cp_v = pltpu.make_async_copy(wqkv_hbm.at[:, pl.ds(2 * D, D)], wv_raw, sem.at[SEM_V])

        def cp_wo(n):
            return pltpu.make_async_copy(wo_hbm.at[:, pl.ds(n * 128, 128)], wo_raw.at[n], sem.at[SEM_V])

        cp_w1 = pltpu.make_async_copy(w1_hbm, w1s, sem.at[SEM_W])
        cp_w3 = pltpu.make_async_copy(w3_hbm, w3s, sem.at[SEM_W])
        cp_w2 = pltpu.make_async_copy(w2_hbm, w2s, sem.at[SEM_W])

        def layernorm(r0, nr, dv=None):
            x = xs[pl.ds(r0, nr), :].astype(f32)
            if dv is not None:
                x = jnp.concatenate([pin(x[:, t * 128:(t + 1) * 128], dv) for t in range(NT)], axis=1)
            m = jnp.mean(x, axis=-1, keepdims=True)
            xc = x - m
            v = jnp.mean(xc * xc, axis=-1, keepdims=True)
            xn[pl.ds(r0, nr), :] = (xc * lax.rsqrt(v + 1e-5)).astype(bf16)

        def pin(val, dv):
            if dv is None:
                return val
            reps = val.shape[0] // dv.shape[0]
            return jnp.where(i < 0, jnp.concatenate([dv] * reps, axis=0), val)

        def perm_cols(src, dst, kt, slot, dv=None):
            k0 = pl.multiple_of(kt * 128, 128)
            for nt in range(NT):
                dvn = None if dv is None else dv[nt * (dv.shape[0] // NT):nt * (dv.shape[0] // NT) + 8, :]
                blk = pin(src[pl.ds(k0, 128), pl.ds(nt * 128, 128)].astype(f32), dvn).T
                for hh in range(4):
                    tsc[slot, pl.ds(PITCH * (4 * nt + hh), 32), :] = blk[32 * hh:32 * hh + 32, :]
            for j in range(NT):
                for dlo in range(4):
                    dst[kt, pl.ds(128 * j + 32 * dlo, 32), :] = (
                        tsc[slot, pl.ds(4 * j + dlo, 32, stride=PITCH), :].astype(bf16))

        def perm_wo_a(kt, slot, y):
            step = y.shape[0] // H
            for h in range(H):
                dv = y[h * step:h * step + 8, :] if pdep else None
                tsc[slot, pl.ds(PITCH * h, 32), :] = pin(wo_raw[kt, pl.ds(32 * h, 32), :].astype(f32), dv)

        def perm_wo_b(kt, slot, y):
            step = y.shape[0] // 32
            for j in range(NT):
                for dlo in range(4):
                    g = 4 * j + dlo
                    dv = y[g * step:g * step + 8, :] if pdep else None
                    wop[kt, pl.ds(128 * j + 32 * dlo, 32), :] = (
                        pin(tsc[slot, pl.ds(4 * j + dlo, 32, stride=PITCH), :], dv).astype(bf16))

        def perm_wo(kt, slot, dv=None):
            for h in range(H):
                tsc[slot, pl.ds(PITCH * h, 32), :] = pin(wo_raw[kt, pl.ds(32 * h, 32), :].astype(f32), dv)
            for j in range(NT):
                for dlo in range(4):
                    wop[kt, pl.ds(128 * j + 32 * dlo, 32), :] = (
                        tsc[slot, pl.ds(4 * j + dlo, 32, stride=PITCH), :].astype(bf16))

        def proj_block(wp, dst, r0, qm, bg, d0=None):
            d0 = r0 if d0 is None else d0
            x_ = xn[pl.ds(r0, qm), :]
            for j in range(NT):
                wt = jnp.concatenate([wp[kt, pl.ds(j * 128, 128), :] for kt in range(NT)], axis=1)
                y = _nt(x_, wt)
                dst[j, pl.ds(d0 + HALO, qm), :] = y
                bg(j, y)

        def attention(p, dv=None):
            r0 = p * AR
            base = pl.multiple_of(i * TM, TM)
            q = [qs[j, pl.ds(base + (HALO + r0), AR), :] for j in range(NT)]
            if dv is not None:
                q = [jnp.where(i < 0, dv, qj) for qj in q]
            logits = []
            for w in range(W):
                acc = None
                for j in range(NT):
                    t_ = q[j] * ks[j, pl.ds(base + (HALO + r0 - DIL * w), AR), :]
                    acc = t_ if acc is None else acc + t_
                acc = acc + pltpu.roll(acc, 64, 1)
                acc = acc + pltpu.roll(acc, 32, 1)
                acc = acc * (DH ** -0.5)
                if r0 < DIL * w:
                    row = i * TM + r0 + lax.broadcasted_iota(jnp.int32, (AR, 128), 0)
                    acc = jnp.where(row >= DIL * w, acc, -1e9)
                logits.append(acc)
            m = logits[0]
            for w in range(1, W):
                m = jnp.maximum(m, logits[w])
            e = [jnp.exp(l - m) for l in logits]
            den = e[0]
            for w in range(1, W):
                den = den + e[w]
            inv = 1.0 / den
            pr = [ew * inv for ew in e]
            for j in range(NT):
                acc = None
                for w in range(W):
                    vb = 0 if vstat else base
                    t_ = pr[w] * vs[j, pl.ds(vb + (HALO + r0 - DIL * w), AR), :]
                    acc = t_ if acc is None else acc + t_
                os_[pl.ds(r0, AR), pl.ds(j * 128, 128)] = acc.astype(bf16)

        def gate_up(x_, c):
            g = _nn(x_, w1s[:, pl.ds(c * FC, FC)])
            u = _nn(x_, w3s[:, pl.ds(c * FC, FC)])
            hv = _silu(g) * u
            hs[:, pl.ds(c * FC, FC)] = hv.astype(bf16)
            return hv[:AR, :128]

        def final_tile(n):
            base = pl.multiple_of(i * TM, TM)
            ffn = _nn(hs[...], w2s[:, pl.ds(n * 128, 128)])
            s = _nn(os_[...], wop[n])
            x_ = xs[pl.ds(base, TM), pl.ds(n * 128, 128)].astype(f32)
            ost[i % 2, :, pl.ds(n * 128, 128)] = (x_ + s * _silu(ffn)).astype(ost.dtype)

        @pl.when(i == 0)
        def _():
            cp_x(0, QM, SEM_X0).start()
            for c in range(NQD):
                cp_q(c).start()
            for g in range(3):
                for cp in cp_group(g):
                    cp.start()
            cp_v.start()
            for kt in range(NT):
                cp_wo(kt).start()
            cp_w1.start(); cp_w3.start(); cp_w2.start()
            for j in range(NT):
                ks[j, pl.ds(0, HALO), :] = jnp.zeros((HALO, 128), f32)
                vs[j, pl.ds(TM if vstat else 0, HALO), :] = jnp.zeros((HALO, 128), f32)
            with sc("waitx0"):
                cp_x(0, QM, SEM_X0).wait()
            with sc("ln0"):
                for r in range(QM // LNR):
                    layernorm(r * LNR, LNR)
            with sc("permq"):
                cpk = NT // NQD

                @pl.loop(0, NQD)
                def _(c):
                    cp_q(c).wait()
                    for kk in range(cpk):
                        perm_cols(wq_raw, wqp, c * cpk + kk, kk % 2)

            @pl.loop(0, NQ)
            @(jax.named_scope("ph1q") if scopes else (lambda f: f))
            def _(rb):
                for g, at in enumerate((0, 1, 3)):
                    @pl.when(rb == at)
                    def _():
                        for cp in cp_group(g):
                            cp.wait()

                rn = pl.multiple_of(((rb + 1) % NQ) * QM, QM)
                nln = QM // LNR

                def bg(j, dv):
                    for r in range(nln):
                        if (r * NT) // nln == j:
                            layernorm(rn + r * LNR, LNR)
                    if j == NT // 2:
                        perm_cols(wk_raw, wkp, rb, 0, dv if qdep else None)

                proj_block(wqp, qs, pl.multiple_of(rb * QM, QM), QM, bg)

            cp_v.wait()
            for kt in range(NT):
                cp_wo(kt).wait()
            if kvm:
                n1 = S // QM1
                kp1 = NT // n1

                @pl.loop(0, n1)
                @(jax.named_scope("ph1kv") if scopes else (lambda f: f))
                def _(rb):
                    r0 = pl.multiple_of(rb * QM1, QM1)
                    proj_block(wkp, ks, r0, QM1, lambda j, dv: perm_cols(wv_raw, wvp, j, j % 2, dv if vdep else None))

                    def bg(j, dv):
                        for kk in range(kp1):
                            if (kk * NT) // kp1 + wa == j:
                                perm_wo_a(rb * kp1 + kk, kk % 2, dv)
                            if (kk * NT) // kp1 + wb == j:
                                perm_wo_b(rb * kp1 + kk, kk % 2, dv)

                    proj_block(wvp, vs, r0, QM1, bg)
            else:
                n1 = S // QM1
                kp1 = NT // n1

                @pl.loop(0, n1)
                @(jax.named_scope("ph1k") if scopes else (lambda f: f))
                def _(rb):
                    def bg(j, dv):
                        for kk in range(kp1):
                            if (kk * NT) // kp1 + (NT // kp1) // 2 == j:
                                perm_cols(wv_raw, wvp, rb * kp1 + kk, kk % 2, dv if kdep else None)

                    proj_block(wkp, ks, pl.multiple_of(rb * QM1, QM1), QM1, bg)

                n2 = S // QM2
                kp2 = NT // n2

                @pl.loop(0, n2)
                @(jax.named_scope("ph1v") if scopes else (lambda f: f))
                def _(rb):
                    def bg(j, dv):
                        for kk in range(kp2):
                            if (kk * NT) // kp2 + wa == j:
                                perm_wo_a(rb * kp2 + kk, kk % 2, dv)
                            if (kk * NT) // kp2 + wb == j:
                                perm_wo_b(rb * kp2 + kk, kk % 2, dv)

                    proj_block(wvp, vs, pl.multiple_of(rb * QM2, QM2), QM2, bg)

            with sc("waitw"):
                cp_w1.wait(); cp_w3.wait(); cp_w2.wait()

        @pl.when(i > 1)
        def _():
            cp_o(i - 2, 0).wait()
            cp_o(i - 2, 1).wait()

        with sc('ph2'):
            base = pl.multiple_of(i * TM, TM)
            x_ = xn[pl.ds(base, TM), :]
            if att_in == 'p2':
                hi = NC if att_hi is None else att_hi
                dv = None
                for c in range(NC):
                    for p in range(NP):
                        if att_lo + (p * (hi - att_lo)) // NP == c:
                            attention(p, dv if dep else None)
                    dv = gate_up(x_, c)
                for n in range(NT):
                    final_tile(n)
                    if n == osplit:
                        cp_o(i, 0).start()
            else:
                dv = None
                for c in range(NC):
                    dv = gate_up(x_, c)
                hi = NT if att_hi is None else att_hi
                for n in range(NT):
                    for p in range(NP):
                        if att_lo + (p * (hi - att_lo)) // NP == n:
                            attention(p, dv if dep else None)
                    g = _silu(_nn(hs[...], w2s[:, pl.ds(n * 128, 128)]))
                    gs[:, pl.ds(n * 128, 128)] = g
                    dv = g[:AR, :]
                for n in range(NT):
                    s_ = _nn(os_[...], wop[n])
                    xr = xs[pl.ds(base, TM), pl.ds(n * 128, 128)].astype(f32)
                    ost[i % 2, :, pl.ds(n * 128, 128)] = (xr + s_ * gs[:, pl.ds(n * 128, 128)]).astype(ost.dtype)
                    if n == osplit:
                        cp_o(i, 0).start()
            cp_o(i, 1).start()

        @pl.when(i == NB - 1)
        def _():
            cp_o(i - 1, 0).wait()
            cp_o(i - 1, 1).wait()
            cp_o(i, 0).wait()
            cp_o(i, 1).wait()

    nsem = 8 + NQD

    def run(x, wqkv, wo, w1, w3, w2):
        x2 = x.reshape(S, D)
        hbm = pl.BlockSpec(memory_space=pl.ANY)
        wp = lambda: pltpu.VMEM((NT, D, 128), bf16)
        out = pl.pallas_call(
            kernel,
            grid=(NB,),
            in_specs=[hbm] * 6,
            out_specs=hbm,
            out_shape=jax.ShapeDtypeStruct((S, D), x.dtype),
            scratch_shapes=[
                pltpu.VMEM((S, D), bf16),
                pltpu.VMEM((S, D), bf16),
                pltpu.VMEM((D, D), bf16),
                pltpu.VMEM((D, D), bf16),
                pltpu.VMEM((D, D), bf16),
                wp(),
                pltpu.VMEM((D, F), bf16),
                pltpu.VMEM((D, F), bf16),
                pltpu.VMEM((F, D), bf16),
                wp(), wp(), wp(), wp(),
                pltpu.VMEM((2, PITCH * H, 128), f32),
                pltpu.VMEM((NT, HALO + S, 128), f32),
                pltpu.VMEM((NT, HALO + S, 128), f32),
                pltpu.VMEM((NT, HALO + (TM if vstat else S), 128), f32),
                pltpu.VMEM((TM, D), bf16),
                pltpu.VMEM((TM, F), bf16),
                pltpu.VMEM((2, TM, D), bf16),
                pltpu.VMEM((TM, D), f32),
                pltpu.SemaphoreType.DMA((nsem,)),
            ],
            compiler_params=pltpu.CompilerParams(
                dimension_semantics=("arbitrary",), vmem_limit_bytes=110 * 1024 * 1024, flags=flags),
        )(x2, wqkv, wo, w1, w3, w2)
        return out.reshape(1, S, D)

    return run


@jax.jit
def pallas_recurrent_scan__sliding_local_dilated__glu_gated_swiglu__prompt_kernel(
    A_x, A_wqkv, A_wo, B_x, B_w1, B_w3, B_w2,
):
    del B_x
    return build()(A_x, A_wqkv, A_wo, B_w1, B_w3, B_w2)
```

```python
import functools

import jax
import jax.numpy as jnp
from jax import lax
from jax.experimental import pallas as pl
from jax.experimental.pallas import tpu as pltpu

f32, bf16 = jnp.float32, jnp.bfloat16

H, DH, W, DIL = 32, 32, 8, 2
LANES = 128
HALO = 16
PITCH = 33
EPS = 1e-5
FLAGS = {"XLA_TPU_EVENLY_DISTRIBUTE_CRITICAL_NODES": True}

_nn = functools.partial(jnp.dot, preferred_element_type=f32)


def _nt(a, b):
    return lax.dot_general(a, b, (((1,), (1,)), ((), ())), preferred_element_type=f32)


def _silu(x):
    hx = 0.5 * x
    return hx * (1.0 + jnp.tanh(hx))


def build(S=2048, F=3584, TM=256, QM=256, KVM=512, FC=128, AR=8, LNR=64, NQD=4,
          att_lo=2, att_hi=None, osplit=5, wa=0, wb=2, flags=FLAGS, interpret=False):
    D = H * DH
    NT = D // LANES
    NB = S // TM
    NQ = S // QM
    NKV = S // KVM
    NC = F // FC
    NP = TM // AR
    OPK = NT // NKV
    att_hi = NC if att_hi is None else att_hi
    assert NQ == NT and NB >= 2
    GROUPS = ((1, 1, 0, 1, 0), (2, 2, 1, 2, 1), (4, 4, 3, 5, 3))
    SEM_X0, SEM_G, SEM_V, SEM_W, SEM_O, SEM_Q = 0, 1, 4, 5, 6, 8
    NSEM = SEM_Q + NQD

    def kernel(x_hbm, wqkv_hbm, wo_hbm, w1_hbm, w3_hbm, w2_hbm, o_hbm,
               xs, xn, wq_raw, wk_raw, wv_raw, wo_raw, w1s, w3s, w2s, wqp, wkp, wvp, wop, tsc,
               qs, ks, vs, os_, hs, ost, sem):
        i = pl.program_id(0)

        def cp_x(r0, nr, s):
            return pltpu.make_async_copy(x_hbm.at[pl.ds(r0, nr), :], xs.at[pl.ds(r0, nr), :], sem.at[s])

        def cp_q(c):
            n = D // NQD
            k0 = pl.multiple_of(c * n, n)
            return pltpu.make_async_copy(
                wqkv_hbm.at[pl.ds(k0, n), pl.ds(0, D)], wq_raw.at[pl.ds(k0, n), :], sem.at[SEM_Q + c])

        def cp_group(g):
            xb, xnb, kb, knb, _ = GROUPS[g]
            rows = pl.ds(kb * LANES, knb * LANES)
            return (cp_x(xb * QM, xnb * QM, SEM_G + g),
                    pltpu.make_async_copy(wqkv_hbm.at[rows, pl.ds(D, D)], wk_raw.at[rows, :], sem.at[SEM_G + g]))

        cps_v = [pltpu.make_async_copy(wqkv_hbm.at[:, pl.ds(2 * D, D)], wv_raw, sem.at[SEM_V])]
        cps_v += [pltpu.make_async_copy(wo_hbm.at[:, pl.ds(n * LANES, LANES)], wo_raw.at[n], sem.at[SEM_V])
                  for n in range(NT)]
        cps_w = [pltpu.make_async_copy(src, dst, sem.at[SEM_W])
                 for src, dst in ((w1_hbm, w1s), (w3_hbm, w3s), (w2_hbm, w2s))]

        def cp_o(step, part):
            split = (osplit + 1) * LANES
            c0, nc = (0, split) if part == 0 else (split, D - split)
            r0 = pl.multiple_of(step * TM, TM)
            return pltpu.make_async_copy(
                ost.at[step % 2, :, pl.ds(c0, nc)], o_hbm.at[pl.ds(r0, TM), pl.ds(c0, nc)],
                sem.at[SEM_O + step % 2])

        def pin(val, dv):
            if dv is None:
                return val
            return jnp.where(i < 0, jnp.concatenate([dv] * (val.shape[0] // dv.shape[0]), axis=0), val)

        def tile_of(y, k, n):
            r = k * (y.shape[0] // n)
            return y[r:r + 8, :]

        def layernorm(r0, nr):
            x = xs[pl.ds(r0, nr), :].astype(f32)
            xc = x - jnp.mean(x, axis=-1, keepdims=True)
            var = jnp.mean(xc * xc, axis=-1, keepdims=True)
            xn[pl.ds(r0, nr), :] = (xc * lax.rsqrt(var + EPS)).astype(bf16)

        def perm_cols(src, dst, kt, slot, y=None):
            k0 = pl.multiple_of(kt * LANES, LANES)
            for nt in range(NT):
                blk = src[pl.ds(k0, LANES), pl.ds(nt * LANES, LANES)].astype(f32)
                blk = pin(blk, None if y is None else tile_of(y, nt, NT)).T
                for hh in range(4):
                    tsc[slot, pl.ds(PITCH * (4 * nt + hh), DH), :] = blk[DH * hh:DH * (hh + 1), :]
            for j in range(NT):
                for d in range(4):
                    dst[kt, pl.ds(LANES * j + H * d, H), :] = (
                        tsc[slot, pl.ds(4 * j + d, H, stride=PITCH), :].astype(bf16))

        def perm_wo_load(kt, slot, y):
            for h in range(H):
                tsc[slot, pl.ds(PITCH * h, DH), :] = pin(
                    wo_raw[kt, pl.ds(DH * h, DH), :].astype(f32), tile_of(y, h, H))

        def perm_wo_store(kt, slot, y):
            for j in range(NT):
                for d in range(4):
                    rows = tsc[slot, pl.ds(4 * j + d, H, stride=PITCH), :]
                    wop[kt, pl.ds(LANES * j + H * d, H), :] = pin(rows, tile_of(y, 4 * j + d, H)).astype(bf16)

        def project(wp, dst, r0, rows, background):
            x_ = xn[pl.ds(r0, rows), :]
            for j in range(NT):
                wt = jnp.concatenate([wp[kt, pl.ds(j * LANES, LANES), :] for kt in range(NT)], axis=1)
                y = _nt(x_, wt)
                dst[j, pl.ds(r0 + HALO, rows), :] = y
                background(j, y)

        def attention(base, p, dv):
            r0 = p * AR
            q = [pin(qs[j, pl.ds(base + (HALO + r0), AR), :], dv) for j in range(NT)]
            logits = []
            for w in range(W):
                acc = None
                for j in range(NT):
                    t = q[j] * ks[j, pl.ds(base + (HALO + r0 - DIL * w), AR), :]
                    acc = t if acc is None else acc + t
                acc = acc + pltpu.roll(acc, 64, 1)
                acc = acc + pltpu.roll(acc, 32, 1)
                acc = acc * (DH ** -0.5)
                if r0 < DIL * w:
                    row = base + r0 + lax.broadcasted_iota(jnp.int32, (AR, LANES), 0)
                    acc = jnp.where(row >= DIL * w, acc, -1e9)
                logits.append(acc)
            m = functools.reduce(jnp.maximum, logits)
            e = [jnp.exp(l - m) for l in logits]
            inv = 1.0 / functools.reduce(jnp.add, e)
            pr = [ew * inv for ew in e]
            for j in range(NT):
                acc = None
                for w in range(W):
                    t = pr[w] * vs[j, pl.ds(base + (HALO + r0 - DIL * w), AR), :]
                    acc = t if acc is None else acc + t
                os_[pl.ds(r0, AR), pl.ds(j * LANES, LANES)] = acc.astype(bf16)

        @pl.when(i == 0)
        def _():
            cp_x(0, QM, SEM_X0).start()
            for c in range(NQD):
                cp_q(c).start()
            for g in range(len(GROUPS)):
                for cp in cp_group(g):
                    cp.start()
            for cp in cps_v + cps_w:
                cp.start()

            for j in range(NT):
                ks[j, pl.ds(0, HALO), :] = jnp.zeros((HALO, LANES), f32)
                vs[j, pl.ds(0, HALO), :] = jnp.zeros((HALO, LANES), f32)

            cp_x(0, QM, SEM_X0).wait()
            for r in range(QM // LNR):
                layernorm(r * LNR, LNR)

            @pl.loop(0, NQD)
            def _(c):
                cp_q(c).wait()
                for kk in range(NT // NQD):
                    perm_cols(wq_raw, wqp, c * (NT // NQD) + kk, kk % 2)

            @pl.loop(0, NQ)
            def _(rb):
                for g, group in enumerate(GROUPS):
                    @pl.when(rb == group[4])
                    def _():
                        for cp in cp_group(g):
                            cp.wait()

                rn = pl.multiple_of(((rb + 1) % NQ) * QM, QM)
                nln = QM // LNR

                def background(j, y):
                    for r in range(nln):
                        if (r * NT) // nln == j:
                            layernorm(rn + r * LNR, LNR)
                    if j == NT // 2:
                        perm_cols(wk_raw, wkp, rb, 0)

                project(wqp, qs, pl.multiple_of(rb * QM, QM), QM, background)

            for cp in cps_v:
                cp.wait()

            @pl.loop(0, NKV)
            def _(rb):
                r0 = pl.multiple_of(rb * KVM, KVM)
                project(wkp, ks, r0, KVM, lambda j, y: perm_cols(wv_raw, wvp, j, j % 2, y))

                def background(j, y):
                    for kk in range(OPK):
                        if (kk * NT) // OPK + wa == j:
                            perm_wo_load(rb * OPK + kk, kk % 2, y)
                        if (kk * NT) // OPK + wb == j:
                            perm_wo_store(rb * OPK + kk, kk % 2, y)

                project(wvp, vs, r0, KVM, background)

            for cp in cps_w:
                cp.wait()

        @pl.when(i >= 2)
        def _():
            cp_o(i - 2, 0).wait()
            cp_o(i - 2, 1).wait()

        base = pl.multiple_of(i * TM, TM)
        x_ = xn[pl.ds(base, TM), :]
        dv = None
        for c in range(NC):
            for p in range(NP):
                if att_lo + (p * (att_hi - att_lo)) // NP == c:
                    attention(base, p, dv)
            cols = pl.ds(c * FC, FC)
            h = _silu(_nn(x_, w1s[:, cols])) * _nn(x_, w3s[:, cols])
            hs[:, cols] = h.astype(bf16)
            dv = h[:AR, :LANES]

        for n in range(NT):
            cols = pl.ds(n * LANES, LANES)
            ffn = _nn(hs[...], w2s[:, cols])
            s = _nn(os_[...], wop[n])
            ost[i % 2, :, cols] = (xs[pl.ds(base, TM), cols].astype(f32) + s * _silu(ffn)).astype(ost.dtype)
            if n == osplit:
                cp_o(i, 0).start()
        cp_o(i, 1).start()

        @pl.when(i == NB - 1)
        def _():
            for step in (i - 1, i):
                cp_o(step, 0).wait()
                cp_o(step, 1).wait()

    def run(x, wqkv, wo, w1, w3, w2):
        hbm = pl.BlockSpec(memory_space=pl.ANY)
        slabs = lambda: pltpu.VMEM((NT, D, LANES), bf16)
        tiles = lambda: pltpu.VMEM((NT, HALO + S, LANES), f32)
        out = pl.pallas_call(
            kernel,
            grid=(NB,),
            in_specs=[hbm] * 6,
            out_specs=hbm,
            out_shape=jax.ShapeDtypeStruct((S, D), x.dtype),
            scratch_shapes=[
                pltpu.VMEM((S, D), bf16),
                pltpu.VMEM((S, D), bf16),
                pltpu.VMEM((D, D), bf16),
                pltpu.VMEM((D, D), bf16),
                pltpu.VMEM((D, D), bf16),
                slabs(),
                pltpu.VMEM((D, F), bf16),
                pltpu.VMEM((D, F), bf16),
                pltpu.VMEM((F, D), bf16),
                slabs(), slabs(), slabs(),
                slabs(),
                pltpu.VMEM((2, PITCH * H + DH, LANES), f32),
                tiles(), tiles(), tiles(),
                pltpu.VMEM((TM, D), bf16),
                pltpu.VMEM((TM, F), bf16),
                pltpu.VMEM((2, TM, D), x.dtype),
                pltpu.SemaphoreType.DMA((NSEM,)),
            ],
            compiler_params=pltpu.CompilerParams(
                dimension_semantics=("arbitrary",), vmem_limit_bytes=110 * 1024 * 1024, flags=flags),
            interpret=interpret,
        )(x.reshape(S, D), wqkv, wo, w1, w3, w2)
        return out.reshape(x.shape)

    return run


@jax.jit
def pallas_recurrent_scan__sliding_local_dilated__glu_gated_swiglu__prompt_kernel(
    A_x: jax.Array,
    A_wqkv: jax.Array,
    A_wo: jax.Array,
    B_x: jax.Array,
    B_w1: jax.Array,
    B_w3: jax.Array,
    B_w2: jax.Array,
):
    del B_x
    return build()(A_x, A_wqkv, A_wo, B_w1, B_w3, B_w2)
```

```python
import functools

import jax
import jax.numpy as jnp
from jax import lax
from jax.experimental import pallas as pl
from jax.experimental.pallas import tpu as pltpu

f32, bf16 = jnp.float32, jnp.bfloat16

H, DH, W, DIL = 32, 32, 8, 2
LANES = 128
HALO = 16
PITCH = 33
EPS = 1e-5
FLAGS = {"XLA_TPU_EVENLY_DISTRIBUTE_CRITICAL_NODES": True}

_nn = functools.partial(jnp.dot, preferred_element_type=f32)


def _nt(a, b):
    return lax.dot_general(a, b, (((1,), (1,)), ((), ())), preferred_element_type=f32)


def _silu(x):
    hx = 0.5 * x
    return hx * (1.0 + jnp.tanh(hx))


def build(S=2048, F=3584, TM=256, QM=256, KVM=512, FC=128, AR=8, LNR=64, NQD=4,
          att_lo=1, att_hi=None, osplit=(6, 7, 8), wa=0, wb=2, vsh=1, flags=FLAGS, interpret=False):
    D = H * DH
    NT = D // LANES
    NB = S // TM
    NQ = S // QM
    NKV = S // KVM
    NC = F // FC
    NP = TM // AR
    OPK = NT // NKV
    att_hi = NC - 2 if att_hi is None else att_hi
    assert NQ == NT and NB >= 2
    GROUPS = ((1, 1, 0, 1, 0), (2, 2, 1, 2, 1), (4, 4, 3, 5, 3))
    SEM_X0, SEM_G, SEM_V, SEM_W, SEM_O, SEM_Q = 0, 1, 4, 5, 6, 8
    NSEM = SEM_Q + NQD

    def kernel(x_hbm, wqkv_hbm, wo_hbm, w1_hbm, w3_hbm, w2_hbm, o_hbm,
               xs, xn, wq_raw, wk_raw, wv_raw, wo_raw, w1s, w3s, w2s, wqp, wkp, wvp, wop, tsc,
               qs, ks, vs, os_, hs, ost, sem):
        i = pl.program_id(0)

        def cp_x(r0, nr, s):
            return pltpu.make_async_copy(x_hbm.at[pl.ds(r0, nr), :], xs.at[pl.ds(r0, nr), :], sem.at[s])

        def cp_q(c):
            n = D // NQD
            k0 = pl.multiple_of(c * n, n)
            return pltpu.make_async_copy(
                wqkv_hbm.at[pl.ds(k0, n), pl.ds(0, D)], wq_raw.at[pl.ds(k0, n), :], sem.at[SEM_Q + c])

        def cp_group(g):
            xb, xnb, kb, knb, _ = GROUPS[g]
            rows = pl.ds(kb * LANES, knb * LANES)
            return (cp_x(xb * QM, xnb * QM, SEM_G + g),
                    pltpu.make_async_copy(wqkv_hbm.at[rows, pl.ds(D, D)], wk_raw.at[rows, :], sem.at[SEM_G + g]))

        cps_v = [pltpu.make_async_copy(wqkv_hbm.at[:, pl.ds(2 * D, D)], wv_raw, sem.at[SEM_V])]
        cps_v += [pltpu.make_async_copy(wo_hbm.at[:, pl.ds(n * LANES, LANES)], wo_raw.at[n], sem.at[SEM_V])
                  for n in range(NT)]
        cps_w = [pltpu.make_async_copy(src, dst, sem.at[SEM_W])
                 for src, dst in ((w1_hbm, w1s), (w3_hbm, w3s), (w2_hbm, w2s))]

        def cp_o(step, part):
            lo = 0 if part == 0 else osplit[part - 1]
            c0, nc = lo * LANES, (osplit[part] - lo) * LANES
            r0 = pl.multiple_of(step * TM, TM)
            return pltpu.make_async_copy(
                ost.at[step % 2, :, pl.ds(c0, nc)], o_hbm.at[pl.ds(r0, TM), pl.ds(c0, nc)],
                sem.at[SEM_O + step % 2])

        def pin(val, dv):
            if dv is None:
                return val
            return jnp.where(i < 0, jnp.concatenate([dv] * (val.shape[0] // dv.shape[0]), axis=0), val)

        def tile_of(y, k, n):
            r = k * (y.shape[0] // n)
            return y[r:r + 8, :]

        def layernorm(r0, nr):
            x = xs[pl.ds(r0, nr), :].astype(f32)
            xc = x - jnp.mean(x, axis=-1, keepdims=True)
            var = jnp.mean(xc * xc, axis=-1, keepdims=True)
            xn[pl.ds(r0, nr), :] = (xc * lax.rsqrt(var + EPS)).astype(bf16)

        def perm_cols(src, dst, kt, slot, y=None):
            k0 = pl.multiple_of(kt * LANES, LANES)
            for nt in range(NT):
                blk = src[pl.ds(k0, LANES), pl.ds(nt * LANES, LANES)].astype(f32)
                blk = pin(blk, None if y is None else tile_of(y, nt, NT)).T
                for hh in range(4):
                    tsc[slot, pl.ds(PITCH * (4 * nt + hh), DH), :] = blk[DH * hh:DH * (hh + 1), :]
            for j in range(NT):
                for d in range(4):
                    dst[kt, pl.ds(LANES * j + H * d, H), :] = (
                        tsc[slot, pl.ds(4 * j + d, H, stride=PITCH), :].astype(bf16))

        def perm_wo_load(kt, slot, y):
            for h in range(H):
                tsc[slot, pl.ds(PITCH * h, DH), :] = pin(
                    wo_raw[kt, pl.ds(DH * h, DH), :].astype(f32), tile_of(y, h, H))

        def perm_wo_store(kt, slot, y):
            for j in range(NT):
                for d in range(4):
                    rows = tsc[slot, pl.ds(4 * j + d, H, stride=PITCH), :]
                    wop[kt, pl.ds(LANES * j + H * d, H), :] = pin(rows, tile_of(y, 4 * j + d, H)).astype(bf16)

        def project(wp, dst, r0, rows, background):
            x_ = xn[pl.ds(r0, rows), :]
            for j in range(NT):
                wt = jnp.concatenate([wp[kt, pl.ds(j * LANES, LANES), :] for kt in range(NT)], axis=1)
                y = _nt(x_, wt)
                dst[j, pl.ds(r0 + HALO, rows), :] = y
                background(j, y)

        def attention(base, p, dv):
            r0 = p * AR
            q = [pin(qs[j, pl.ds(base + (HALO + r0), AR), :], dv) for j in range(NT)]
            logits = []
            for w in range(W):
                acc = None
                for j in range(NT):
                    t = q[j] * ks[j, pl.ds(base + (HALO + r0 - DIL * w), AR), :]
                    acc = t if acc is None else acc + t
                acc = acc + pltpu.roll(acc, 64, 1)
                acc = acc + pltpu.roll(acc, 32, 1)
                acc = acc * (DH ** -0.5)
                if r0 < DIL * w:
                    row = base + r0 + lax.broadcasted_iota(jnp.int32, (AR, LANES), 0)
                    acc = jnp.where(row >= DIL * w, acc, -1e9)
                logits.append(acc)
            m = functools.reduce(jnp.maximum, logits)
            e = [jnp.exp(l - m) for l in logits]
            inv = 1.0 / functools.reduce(jnp.add, e)
            pr = [ew * inv for ew in e]
            for j in range(NT):
                acc = None
                for w in range(W):
                    t = pr[w] * vs[j, pl.ds(base + (HALO + r0 - DIL * w), AR), :]
                    acc = t if acc is None else acc + t
                os_[pl.ds(r0, AR), pl.ds(j * LANES, LANES)] = acc.astype(bf16)

        @pl.when(i == 0)
        def _():
            cp_x(0, QM, SEM_X0).start()
            for c in range(NQD):
                cp_q(c).start()
            for g in range(len(GROUPS)):
                for cp in cp_group(g):
                    cp.start()
            for cp in cps_v + cps_w:
                cp.start()

            for j in range(NT):
                ks[j, pl.ds(0, HALO), :] = jnp.zeros((HALO, LANES), f32)
                vs[j, pl.ds(0, HALO), :] = jnp.zeros((HALO, LANES), f32)

            cp_x(0, QM, SEM_X0).wait()
            for r in range(QM // LNR):
                layernorm(r * LNR, LNR)

            @pl.loop(0, NQD)
            def _(c):
                cp_q(c).wait()
                for kk in range(NT // NQD):
                    perm_cols(wq_raw, wqp, c * (NT // NQD) + kk, kk % 2)

            @pl.loop(0, NQ)
            def _(rb):
                for g, group in enumerate(GROUPS):
                    @pl.when(rb == group[4])
                    def _():
                        for cp in cp_group(g):
                            cp.wait()

                rn = pl.multiple_of(((rb + 1) % NQ) * QM, QM)
                nln = QM // LNR

                def background(j, y):
                    for r in range(nln):
                        if (r * NT) // nln == j:
                            layernorm(rn + r * LNR, LNR)
                    if j == NT // 2:
                        perm_cols(wk_raw, wkp, rb, 0)

                project(wqp, qs, pl.multiple_of(rb * QM, QM), QM, background)

            for cp in cps_v:
                cp.wait()

            @pl.loop(0, NKV)
            def _(rb):
                r0 = pl.multiple_of(rb * KVM, KVM)
                def perm_v(j, y):
                    for c in range(NT):
                        if max(c - vsh, 0) == j:
                            perm_cols(wv_raw, wvp, c, c % 2, y)

                project(wkp, ks, r0, KVM, perm_v)

                def background(j, y):
                    for kk in range(OPK):
                        if (kk * NT) // OPK + wa == j:
                            perm_wo_load(rb * OPK + kk, kk % 2, y)
                        if (kk * NT) // OPK + wb == j:
                            perm_wo_store(rb * OPK + kk, kk % 2, y)

                project(wvp, vs, r0, KVM, background)

            for cp in cps_w:
                cp.wait()

        @pl.when(i >= 2)
        def _():
            for part in range(len(osplit)):
                cp_o(i - 2, part).wait()

        base = pl.multiple_of(i * TM, TM)
        x_ = xn[pl.ds(base, TM), :]
        dv = None
        for c in range(NC):
            for p in range(NP):
                if att_lo + (p * (att_hi - att_lo)) // NP == c:
                    attention(base, p, dv)
            cols = pl.ds(c * FC, FC)
            h = _silu(_nn(x_, w1s[:, cols])) * _nn(x_, w3s[:, cols])
            hs[:, cols] = h.astype(bf16)
            dv = h[:AR, :LANES]

        for n in range(NT):
            cols = pl.ds(n * LANES, LANES)
            ffn = _nn(hs[...], w2s[:, cols])
            s = _nn(os_[...], wop[n])
            ost[i % 2, :, cols] = (xs[pl.ds(base, TM), cols].astype(f32) + s * _silu(ffn)).astype(ost.dtype)
            if n + 1 in osplit:
                cp_o(i, osplit.index(n + 1)).start()

        @pl.when(i == NB - 1)
        def _():
            for step in (i - 1, i):
                for part in range(len(osplit)):
                    cp_o(step, part).wait()

    def run(x, wqkv, wo, w1, w3, w2):
        hbm = pl.BlockSpec(memory_space=pl.ANY)
        slabs = lambda: pltpu.VMEM((NT, D, LANES), bf16)
        tiles = lambda: pltpu.VMEM((NT, HALO + S, LANES), f32)
        out = pl.pallas_call(
            kernel,
            grid=(NB,),
            in_specs=[hbm] * 6,
            out_specs=hbm,
            out_shape=jax.ShapeDtypeStruct((S, D), x.dtype),
            scratch_shapes=[
                pltpu.VMEM((S, D), bf16),
                pltpu.VMEM((S, D), bf16),
                pltpu.VMEM((D, D), bf16),
                pltpu.VMEM((D, D), bf16),
                pltpu.VMEM((D, D), bf16),
                slabs(),
                pltpu.VMEM((D, F), bf16),
                pltpu.VMEM((D, F), bf16),
                pltpu.VMEM((F, D), bf16),
                slabs(), slabs(), slabs(),
                slabs(),
                pltpu.VMEM((2, PITCH * H + DH, LANES), f32),
                tiles(), tiles(), tiles(),
                pltpu.VMEM((TM, D), bf16),
                pltpu.VMEM((TM, F), bf16),
                pltpu.VMEM((2, TM, D), x.dtype),
                pltpu.SemaphoreType.DMA((NSEM,)),
            ],
            compiler_params=pltpu.CompilerParams(
                dimension_semantics=("arbitrary",), vmem_limit_bytes=110 * 1024 * 1024, flags=flags),
            interpret=interpret,
        )(x.reshape(S, D), wqkv, wo, w1, w3, w2)
        return out.reshape(x.shape)

    return run


@jax.jit
def pallas_recurrent_scan__sliding_local_dilated__glu_gated_swiglu__prompt_kernel(
    A_x: jax.Array,
    A_wqkv: jax.Array,
    A_wo: jax.Array,
    B_x: jax.Array,
    B_w1: jax.Array,
    B_w3: jax.Array,
    B_w2: jax.Array,
):
    del B_x
    return build()(A_x, A_wqkv, A_wo, B_w1, B_w3, B_w2)
```

```python
import functools

import jax
import jax.numpy as jnp
from jax import lax
from jax.experimental import pallas as pl
from jax.experimental.pallas import tpu as pltpu

f32, bf16 = jnp.float32, jnp.bfloat16

H, DH, W, DIL = 32, 32, 8, 2
LANES = 128
HALO = 16
PITCH = 33
EPS = 1e-5
FLAGS = {"XLA_TPU_EVENLY_DISTRIBUTE_CRITICAL_NODES": True}

_nn = functools.partial(jnp.dot, preferred_element_type=f32)


def _nt(a, b):
    return lax.dot_general(a, b, (((1,), (1,)), ((), ())), preferred_element_type=f32)


def _silu(x):
    hx = 0.5 * x
    return hx * (1.0 + jnp.tanh(hx))


def build(S=2048, F=3584, TM=256, QM=256, KVM=512, FC=128, AR=8, LNR=64, NQD=4,
          att_lo=1, att_hi=None, osplit=(6, 7, 8), wa=0, wb=2, vsh=1, flags=FLAGS, interpret=False):
    D = H * DH
    NT = D // LANES
    NB = S // TM
    NQ = S // QM
    NKV = S // KVM
    NC = F // FC
    NP = TM // AR
    OPK = NT // NKV
    att_hi = NC - 2 if att_hi is None else att_hi
    assert NQ == NT and NB >= 2
    assert 0 <= att_lo < NC and att_lo < att_hi <= NC
    GROUPS = ((1, 1, 0, 1, 0), (2, 2, 1, 2, 1), (4, 4, 3, 5, 3))
    SEM_X0, SEM_G, SEM_V, SEM_W, SEM_O, SEM_Q = 0, 1, 4, 5, 6, 8
    NSEM = SEM_Q + NQD

    def kernel(x_hbm, wqkv_hbm, wo_hbm, w1_hbm, w3_hbm, w2_hbm, o_hbm,
               xs, xn, wq_raw, wk_raw, wv_raw, wo_raw, w1s, w3s, w2s, wqp, wkp, wvp, wop, tsc,
               qs, ks, vs, os_, hs, ost, sem):
        i = pl.program_id(0)

        def cp_x(r0, nr, s):
            return pltpu.make_async_copy(x_hbm.at[pl.ds(r0, nr), :], xs.at[pl.ds(r0, nr), :], sem.at[s])

        def cp_q(c):
            n = D // NQD
            k0 = pl.multiple_of(c * n, n)
            return pltpu.make_async_copy(
                wqkv_hbm.at[pl.ds(k0, n), pl.ds(0, D)], wq_raw.at[pl.ds(k0, n), :], sem.at[SEM_Q + c])

        def cp_group(g):
            xb, xnb, kb, knb, _ = GROUPS[g]
            rows = pl.ds(kb * LANES, knb * LANES)
            return (cp_x(xb * QM, xnb * QM, SEM_G + g),
                    pltpu.make_async_copy(wqkv_hbm.at[rows, pl.ds(D, D)], wk_raw.at[rows, :], sem.at[SEM_G + g]))

        cps_v = [pltpu.make_async_copy(wqkv_hbm.at[:, pl.ds(2 * D, D)], wv_raw, sem.at[SEM_V])]
        cps_v += [pltpu.make_async_copy(wo_hbm.at[:, pl.ds(n * LANES, LANES)], wo_raw.at[n], sem.at[SEM_V])
                  for n in range(NT)]
        cps_w = [pltpu.make_async_copy(src, dst, sem.at[SEM_W])
                 for src, dst in ((w1_hbm, w1s), (w3_hbm, w3s), (w2_hbm, w2s))]

        def cp_o(step, part):
            lo = 0 if part == 0 else osplit[part - 1]
            c0, nc = lo * LANES, (osplit[part] - lo) * LANES
            r0 = pl.multiple_of(step * TM, TM)
            return pltpu.make_async_copy(
                ost.at[step & 1, :, pl.ds(c0, nc)], o_hbm.at[pl.ds(r0, TM), pl.ds(c0, nc)],
                sem.at[SEM_O + (step & 1)])

        def pin(val, dv):
            if dv is None:
                return val
            return jnp.where(i < 0, jnp.concatenate([dv] * (val.shape[0] // dv.shape[0]), axis=0), val)

        def tile_of(y, k, n):
            r = k * (y.shape[0] // n)
            return y[r:r + 8, :]

        def layernorm(r0, nr):
            x = xs[pl.ds(r0, nr), :].astype(f32)
            xc = x - jnp.mean(x, axis=-1, keepdims=True)
            var = jnp.mean(xc * xc, axis=-1, keepdims=True)
            xn[pl.ds(r0, nr), :] = (xc * lax.rsqrt(var + EPS)).astype(bf16)

        def perm_cols(src, dst, kt, slot, y=None):
            k0 = pl.multiple_of(kt * LANES, LANES)
            for nt in range(NT):
                blk = src[pl.ds(k0, LANES), pl.ds(nt * LANES, LANES)].astype(f32)
                blk = pin(blk, None if y is None else tile_of(y, nt, NT)).T
                for hh in range(4):
                    tsc[slot, pl.ds(PITCH * (4 * nt + hh), DH), :] = blk[DH * hh:DH * (hh + 1), :]
            for j in range(NT):
                for d in range(4):
                    dst[kt, pl.ds(LANES * j + H * d, H), :] = (
                        tsc[slot, pl.ds(4 * j + d, H, stride=PITCH), :].astype(bf16))

        def perm_wo_load(kt, slot, y):
            for h in range(H):
                tsc[slot, pl.ds(PITCH * h, DH), :] = pin(
                    wo_raw[kt, pl.ds(DH * h, DH), :].astype(f32), tile_of(y, h, H))

        def perm_wo_store(kt, slot, y):
            for j in range(NT):
                for d in range(4):
                    rows = tsc[slot, pl.ds(4 * j + d, H, stride=PITCH), :]
                    wop[kt, pl.ds(LANES * j + H * d, H), :] = pin(rows, tile_of(y, 4 * j + d, H)).astype(bf16)

        def project(wp, dst, r0, rows, background):
            x_ = xn[pl.ds(r0, rows), :]
            for j in range(NT):
                wt = jnp.concatenate([wp[kt, pl.ds(j * LANES, LANES), :] for kt in range(NT)], axis=1)
                y = _nt(x_, wt)
                dst[j, pl.ds(r0 + HALO, rows), :] = y
                background(j, y)

        def attention(base, p, dv):
            r0 = p * AR
            q = [pin(qs[j, pl.ds(base + (HALO + r0), AR), :], dv) for j in range(NT)]
            logits = []
            for w in range(W):
                acc = None
                for j in range(NT):
                    t = q[j] * ks[j, pl.ds(base + (HALO + r0 - DIL * w), AR), :]
                    acc = t if acc is None else acc + t
                acc = acc + pltpu.roll(acc, 64, 1)
                acc = acc + pltpu.roll(acc, 32, 1)
                acc = acc * (DH ** -0.5)
                if r0 < DIL * w:
                    row = base + r0 + lax.broadcasted_iota(jnp.int32, (AR, LANES), 0)
                    acc = jnp.where(row >= DIL * w, acc, -1e9)
                logits.append(acc)
            m = functools.reduce(jnp.maximum, logits)
            e = [jnp.exp(l - m) for l in logits]
            inv = 1.0 / functools.reduce(jnp.add, e)
            pr = [ew * inv for ew in e]
            for j in range(NT):
                acc = None
                for w in range(W):
                    t = pr[w] * vs[j, pl.ds(base + (HALO + r0 - DIL * w), AR), :]
                    acc = t if acc is None else acc + t
                os_[pl.ds(r0, AR), pl.ds(j * LANES, LANES)] = acc.astype(bf16)

        @pl.when(i == 0)
        def _():
            cp_x(0, QM, SEM_X0).start()
            for c in range(NQD):
                cp_q(c).start()
            for g in range(len(GROUPS)):
                for cp in cp_group(g):
                    cp.start()
            for cp in cps_v + cps_w:
                cp.start()

            for j in range(NT):
                for ref in (qs, ks, vs):
                    ref[j, pl.ds(0, HALO), :] = jnp.zeros((HALO, LANES), f32)
            tsc[...] = jnp.zeros(tsc.shape, f32)

            cp_x(0, QM, SEM_X0).wait()
            for r in range(QM // LNR):
                layernorm(r * LNR, LNR)

            @pl.loop(0, NQD)
            def _(c):
                cp_q(c).wait()
                for kk in range(NT // NQD):
                    perm_cols(wq_raw, wqp, c * (NT // NQD) + kk, kk % 2)

            @pl.loop(0, NQ)
            def _(rb):
                for g, group in enumerate(GROUPS):
                    @pl.when(rb == group[4])
                    def _():
                        for cp in cp_group(g):
                            cp.wait()

                rn = pl.multiple_of(((rb + 1) % NQ) * QM, QM)
                nln = QM // LNR

                def background(j, y):
                    for r in range(nln):
                        if (r * NT) // nln == j:
                            layernorm(rn + r * LNR, LNR)
                    if j == NT // 2:
                        perm_cols(wk_raw, wkp, rb, 0)

                project(wqp, qs, pl.multiple_of(rb * QM, QM), QM, background)

            for cp in cps_v:
                cp.wait()

            @pl.loop(0, NKV)
            def _(rb):
                r0 = pl.multiple_of(rb * KVM, KVM)
                def perm_v(j, y):
                    for c in range(NT):
                        if max(c - vsh, 0) == j:
                            perm_cols(wv_raw, wvp, c, c % 2, y)

                project(wkp, ks, r0, KVM, perm_v)

                def background(j, y):
                    for kk in range(OPK):
                        if (kk * NT) // OPK + wa == j:
                            perm_wo_load(rb * OPK + kk, kk % 2, y)
                        if (kk * NT) // OPK + wb == j:
                            perm_wo_store(rb * OPK + kk, kk % 2, y)

                project(wvp, vs, r0, KVM, background)

            for cp in cps_w:
                cp.wait()

        base = pl.multiple_of(i * TM, TM)
        x_ = xn[pl.ds(base, TM), :]
        dv = None
        for c in range(NC):
            for p in range(NP):
                if att_lo + (p * (att_hi - att_lo)) // NP == c:
                    attention(base, p, dv)
            cols = pl.ds(c * FC, FC)
            h = _silu(_nn(x_, w1s[:, cols])) * _nn(x_, w3s[:, cols])
            hs[:, cols] = h.astype(bf16)
            dv = h[:AR, :LANES]

        for n in range(NT):
            cols = pl.ds(n * LANES, LANES)
            ffn = _nn(hs[...], w2s[:, cols])
            s = _nn(os_[...], wop[n])
            ost[i & 1, :, cols] = (xs[pl.ds(base, TM), cols].astype(f32) + s * _silu(ffn)).astype(ost.dtype)
            if n + 1 in osplit:
                cp_o(i, osplit.index(n + 1)).start()

        @pl.when(i >= 1)
        def _():
            for part in range(len(osplit)):
                cp_o(i - 1, part).wait()

        @pl.when(i == NB - 1)
        def _():
            for part in range(len(osplit)):
                cp_o(i, part).wait()

    def run(x, wqkv, wo, w1, w3, w2):
        hbm = pl.BlockSpec(memory_space=pl.ANY)
        slabs = lambda: pltpu.VMEM((NT, D, LANES), bf16)
        tiles = lambda: pltpu.VMEM((NT, HALO + S, LANES), f32)
        out = pl.pallas_call(
            kernel,
            grid=(NB,),
            in_specs=[hbm] * 6,
            out_specs=hbm,
            out_shape=jax.ShapeDtypeStruct((S, D), x.dtype),
            scratch_shapes=[
                pltpu.VMEM((S, D), bf16),
                pltpu.VMEM((S, D), bf16),
                pltpu.VMEM((D, D), bf16),
                pltpu.VMEM((D, D), bf16),
                pltpu.VMEM((D, D), bf16),
                slabs(),
                pltpu.VMEM((D, F), bf16),
                pltpu.VMEM((D, F), bf16),
                pltpu.VMEM((F, D), bf16),
                slabs(), slabs(), slabs(),
                slabs(),
                pltpu.VMEM((2, PITCH * H + DH, LANES), f32),
                tiles(), tiles(), tiles(),
                pltpu.VMEM((TM, D), bf16),
                pltpu.VMEM((TM, F), bf16),
                pltpu.VMEM((2, TM, D), x.dtype),
                pltpu.SemaphoreType.DMA((NSEM,)),
            ],
            compiler_params=pltpu.CompilerParams(
                dimension_semantics=("arbitrary",), vmem_limit_bytes=110 * 1024 * 1024, flags=flags),
            interpret=interpret,
        )(x.reshape(S, D), wqkv, wo, w1, w3, w2)
        return out.reshape(x.shape)

    return run


@jax.jit
def pallas_recurrent_scan__sliding_local_dilated__glu_gated_swiglu__prompt_kernel(
    A_x: jax.Array,
    A_wqkv: jax.Array,
    A_wo: jax.Array,
    B_x: jax.Array,
    B_w1: jax.Array,
    B_w3: jax.Array,
    B_w2: jax.Array,
):
    del B_x
    return build()(A_x, A_wqkv, A_wo, B_w1, B_w3, B_w2)
```

```python
import functools

import jax
import jax.numpy as jnp
from jax import lax
from jax.experimental import pallas as pl
from jax.experimental.pallas import tpu as pltpu

f32, bf16 = jnp.float32, jnp.bfloat16

H, DH, W, DIL = 32, 32, 8, 2
LANES = 128
HALO = 16
PITCH = 33
EPS = 1e-5
FLAGS = {"XLA_TPU_EVENLY_DISTRIBUTE_CRITICAL_NODES": True}

_nn = functools.partial(jnp.dot, preferred_element_type=f32)


def _nt(a, b):
    return lax.dot_general(a, b, (((1,), (1,)), ((), ())), preferred_element_type=f32)


def _silu(x):
    hx = 0.5 * x
    return hx * (1.0 + jnp.tanh(hx))


def build(S=2048, F=3584, TM=256, QM=256, KVM=512, FC=128, AR=8, LNR=64, NQD=4,
          att_lo=1, att_hi=None, osplit=(6, 7, 8), wa=0, wb=2, vsh=1, flags=FLAGS, interpret=False, peel=5):
    D = H * DH
    NT = D // LANES
    NB = S // TM
    NQ = S // QM
    NKV = S // KVM
    NC = F // FC
    NP = TM // AR
    OPK = NT // NKV
    att_hi = NC - 2 if att_hi is None else att_hi
    assert NQ == NT and NB >= 2 and NT // NQD == 2
    assert 0 <= att_lo < NC and att_lo < att_hi <= NC
    GROUPS = ((1, 1, 0, 1, 0), (2, 2, 1, 2, 1), (4, 4, 3, 5, 3))
    SEM_X0, SEM_G, SEM_V, SEM_W, SEM_O, SEM_Q = 0, 1, 4, 5, 6, 8
    NSEM = SEM_Q + NQD + 1

    def kernel(x_hbm, wqkv_hbm, wo_hbm, w1_hbm, w3_hbm, w2_hbm, o_hbm,
               xs, xn, wq_raw, wk_raw, wv_raw, wo_raw, w1s, w3s, w2s, wqp, wkp, wvp, wop, tsc,
               qs, ks, vs, os_, hs, ost, sem):
        i = pl.program_id(0)

        def cp_x(r0, nr, s):
            return pltpu.make_async_copy(x_hbm.at[pl.ds(r0, nr), :], xs.at[pl.ds(r0, nr), :], sem.at[s])

        def cp_q(c):
            n = D // NQD
            k0 = pl.multiple_of(c * n, n)
            return pltpu.make_async_copy(
                wqkv_hbm.at[pl.ds(k0, n), pl.ds(0, D)], wq_raw.at[pl.ds(k0, n), :], sem.at[SEM_Q + c])

        def cp_q_tail(t):
            rows = pl.ds(D - (2 - t) * LANES, LANES)
            return pltpu.make_async_copy(
                wqkv_hbm.at[rows, pl.ds(0, D)], wq_raw.at[rows, :], sem.at[SEM_Q + NQD - 1 + t])

        def cp_group(g):
            xb, xnb, kb, knb, _ = GROUPS[g]
            rows = pl.ds(kb * LANES, knb * LANES)
            return (cp_x(xb * QM, xnb * QM, SEM_G + g),
                    pltpu.make_async_copy(wqkv_hbm.at[rows, pl.ds(D, D)], wk_raw.at[rows, :], sem.at[SEM_G + g]))

        cps_v = [pltpu.make_async_copy(wqkv_hbm.at[:, pl.ds(2 * D, D)], wv_raw, sem.at[SEM_V])]
        cps_v += [pltpu.make_async_copy(wo_hbm.at[:, pl.ds(n * LANES, LANES)], wo_raw.at[n], sem.at[SEM_V])
                  for n in range(NT)]
        cps_w = [pltpu.make_async_copy(src, dst, sem.at[SEM_W])
                 for src, dst in ((w1_hbm, w1s), (w3_hbm, w3s), (w2_hbm, w2s))]

        def cp_o(step, part):
            lo = 0 if part == 0 else osplit[part - 1]
            c0, nc = lo * LANES, (osplit[part] - lo) * LANES
            r0 = pl.multiple_of(step * TM, TM)
            return pltpu.make_async_copy(
                ost.at[step & 1, :, pl.ds(c0, nc)], o_hbm.at[pl.ds(r0, TM), pl.ds(c0, nc)],
                sem.at[SEM_O + (step & 1)])

        def pin(val, dv):
            if dv is None:
                return val
            return jnp.where(i < 0, jnp.concatenate([dv] * (val.shape[0] // dv.shape[0]), axis=0), val)

        def tile_of(y, k, n):
            r = k * (y.shape[0] // n)
            return y[r:r + 8, :]

        def layernorm(r0, nr):
            x = xs[pl.ds(r0, nr), :].astype(f32)
            xc = x - jnp.mean(x, axis=-1, keepdims=True)
            var = jnp.mean(xc * xc, axis=-1, keepdims=True)
            xn[pl.ds(r0, nr), :] = (xc * lax.rsqrt(var + EPS)).astype(bf16)

        def perm_cols(src, dst, kt, slot, y=None):
            k0 = pl.multiple_of(kt * LANES, LANES)
            for nt in range(NT):
                blk = src[pl.ds(k0, LANES), pl.ds(nt * LANES, LANES)].astype(f32)
                blk = pin(blk, None if y is None else tile_of(y, nt, NT)).T
                for hh in range(4):
                    tsc[slot, pl.ds(PITCH * (4 * nt + hh), DH), :] = blk[DH * hh:DH * (hh + 1), :]
            for j in range(NT):
                for d in range(4):
                    dst[kt, pl.ds(LANES * j + H * d, H), :] = (
                        tsc[slot, pl.ds(4 * j + d, H, stride=PITCH), :].astype(bf16))

        def perm_wo_load(kt, slot, y):
            for h in range(H):
                tsc[slot, pl.ds(PITCH * h, DH), :] = pin(
                    wo_raw[kt, pl.ds(DH * h, DH), :].astype(f32), tile_of(y, h, H))

        def perm_wo_store(kt, slot, y):
            for j in range(NT):
                for d in range(4):
                    rows = tsc[slot, pl.ds(4 * j + d, H, stride=PITCH), :]
                    wop[kt, pl.ds(LANES * j + H * d, H), :] = pin(rows, tile_of(y, 4 * j + d, H)).astype(bf16)

        def project(wp, dst, r0, rows, background):
            x_ = xn[pl.ds(r0, rows), :]
            for j in range(NT):
                wt = jnp.concatenate([wp[kt, pl.ds(j * LANES, LANES), :] for kt in range(NT)], axis=1)
                y = _nt(x_, wt)
                dst[j, pl.ds(r0 + HALO, rows), :] = y
                background(j, y)

        def attention(base, p, dv):
            r0 = p * AR
            q = [pin(qs[j, pl.ds(base + (HALO + r0), AR), :], dv) for j in range(NT)]
            logits = []
            for w in range(W):
                acc = None
                for j in range(NT):
                    t = q[j] * ks[j, pl.ds(base + (HALO + r0 - DIL * w), AR), :]
                    acc = t if acc is None else acc + t
                acc = acc + pltpu.roll(acc, 64, 1)
                acc = acc + pltpu.roll(acc, 32, 1)
                acc = acc * (DH ** -0.5)
                if r0 < DIL * w:
                    row = base + r0 + lax.broadcasted_iota(jnp.int32, (AR, LANES), 0)
                    acc = jnp.where(row >= DIL * w, acc, -1e9)
                logits.append(acc)
            m = functools.reduce(jnp.maximum, logits)
            e = [jnp.exp(l - m) for l in logits]
            inv = 1.0 / functools.reduce(jnp.add, e)
            pr = [ew * inv for ew in e]
            for j in range(NT):
                acc = None
                for w in range(W):
                    t = pr[w] * vs[j, pl.ds(base + (HALO + r0 - DIL * w), AR), :]
                    acc = t if acc is None else acc + t
                os_[pl.ds(r0, AR), pl.ds(j * LANES, LANES)] = acc.astype(bf16)

        @pl.when(i == 0)
        def _():
            cp_x(0, QM, SEM_X0).start()
            for c in range(NQD - 1):
                cp_q(c).start()
            cp_q_tail(0).start()
            cp_q_tail(1).start()
            for g in range(len(GROUPS)):
                for cp in cp_group(g):
                    cp.start()
            for cp in cps_v + cps_w:
                cp.start()

            for j in range(NT):
                for ref in (qs, ks, vs):
                    ref[j, pl.ds(0, HALO), :] = jnp.zeros((HALO, LANES), f32)

            @pl.loop(0, tsc.shape[1] // 64)
            def _(r):
                tsc[:, pl.ds(pl.multiple_of(r * 64, 64), 64), :] = jnp.zeros((2, 64, LANES), f32)

            cp_x(0, QM, SEM_X0).wait()
            pl.loop(0, QM // LNR)(lambda r: layernorm(pl.multiple_of(r * LNR, LNR), LNR))

            @pl.loop(0, NQD - 1)
            def _(c):
                cp_q(c).wait()
                for kk in range(NT // NQD):
                    perm_cols(wq_raw, wqp, c * (NT // NQD) + kk, kk % 2)

            for t in range(2):
                cp_q_tail(t).wait()
                perm_cols(wq_raw, wqp, NT - 2 + t, t)

            def q_background(rb, rn, j0):
                nln = QM // LNR

                def background(j, y):
                    for r in range(nln):
                        if j0 + (r * (NT - j0)) // nln == j:
                            layernorm(rn + r * LNR, LNR)
                    if j == (NT + j0) // 2:
                        perm_cols(wk_raw, wkp, rb, 0)

                return background

            bg0 = q_background(0, QM, peel)

            def first(j, y):
                if j == peel - 1:
                    for cp in cp_group(0):
                        cp.wait()
                if j >= peel:
                    bg0(j, y)

            project(wqp, qs, 0, QM, first)

            @pl.loop(1, NQ)
            def _(rb):
                for g, group in enumerate(GROUPS):
                    if g > 0:
                        @pl.when(rb == group[4])
                        def _():
                            for cp in cp_group(g):
                                cp.wait()

                rn = pl.multiple_of(((rb + 1) % NQ) * QM, QM)
                project(wqp, qs, pl.multiple_of(rb * QM, QM), QM, q_background(rb, rn, 0))

            for cp in cps_v:
                cp.wait()

            @pl.loop(0, NKV)
            def _(rb):
                r0 = pl.multiple_of(rb * KVM, KVM)
                def perm_v(j, y):
                    for c in range(NT):
                        if max(c - vsh, 0) == j:
                            perm_cols(wv_raw, wvp, c, c % 2, y)

                project(wkp, ks, r0, KVM, perm_v)

                def background(j, y):
                    for kk in range(OPK):
                        if (kk * NT) // OPK + wa == j:
                            perm_wo_load(rb * OPK + kk, kk % 2, y)
                        if (kk * NT) // OPK + wb == j:
                            perm_wo_store(rb * OPK + kk, kk % 2, y)

                project(wvp, vs, r0, KVM, background)

            for cp in cps_w:
                cp.wait()

        base = pl.multiple_of(i * TM, TM)
        x_ = xn[pl.ds(base, TM), :]
        dv = None
        for c in range(NC):
            for p in range(NP):
                if att_lo + (p * (att_hi - att_lo)) // NP == c:
                    attention(base, p, dv)
            cols = pl.ds(c * FC, FC)
            h = _silu(_nn(x_, w1s[:, cols])) * _nn(x_, w3s[:, cols])
            hs[:, cols] = h.astype(bf16)
            dv = h[:AR, :LANES]

        for n in range(NT):
            cols = pl.ds(n * LANES, LANES)
            ffn = _nn(hs[...], w2s[:, cols])
            s = _nn(os_[...], wop[n])
            ost[i & 1, :, cols] = (xs[pl.ds(base, TM), cols].astype(f32) + s * _silu(ffn)).astype(ost.dtype)
            if n + 1 in osplit:
                cp_o(i, osplit.index(n + 1)).start()

        @pl.when(i >= 1)
        def _():
            for part in range(len(osplit)):
                cp_o(i - 1, part).wait()

        @pl.when(i == NB - 1)
        def _():
            for part in range(len(osplit)):
                cp_o(i, part).wait()

    def run(x, wqkv, wo, w1, w3, w2):
        hbm = pl.BlockSpec(memory_space=pl.ANY)
        slabs = lambda: pltpu.VMEM((NT, D, LANES), bf16)
        tiles = lambda: pltpu.VMEM((NT, HALO + S, LANES), f32)
        out = pl.pallas_call(
            kernel,
            grid=(NB,),
            in_specs=[hbm] * 6,
            out_specs=hbm,
            out_shape=jax.ShapeDtypeStruct((S, D), x.dtype),
            scratch_shapes=[
                pltpu.VMEM((S, D), bf16),
                pltpu.VMEM((S, D), bf16),
                pltpu.VMEM((D, D), bf16),
                pltpu.VMEM((D, D), bf16),
                pltpu.VMEM((D, D), bf16),
                slabs(),
                pltpu.VMEM((D, F), bf16),
                pltpu.VMEM((D, F), bf16),
                pltpu.VMEM((F, D), bf16),
                slabs(), slabs(), slabs(),
                slabs(),
                pltpu.VMEM((2, PITCH * H + DH, LANES), f32),
                tiles(), tiles(), tiles(),
                pltpu.VMEM((TM, D), bf16),
                pltpu.VMEM((TM, F), bf16),
                pltpu.VMEM((2, TM, D), x.dtype),
                pltpu.SemaphoreType.DMA((NSEM,)),
            ],
            compiler_params=pltpu.CompilerParams(
                dimension_semantics=("arbitrary",), vmem_limit_bytes=110 * 1024 * 1024, flags=flags),
            interpret=interpret,
        )(x.reshape(S, D), wqkv, wo, w1, w3, w2)
        return out.reshape(x.shape)

    return run


@jax.jit
def pallas_recurrent_scan__sliding_local_dilated__glu_gated_swiglu__prompt_kernel(
    A_x: jax.Array,
    A_wqkv: jax.Array,
    A_wo: jax.Array,
    B_x: jax.Array,
    B_w1: jax.Array,
    B_w3: jax.Array,
    B_w2: jax.Array,
):
    del B_x
    return build()(A_x, A_wqkv, A_wo, B_w1, B_w3, B_w2)
```
